```python
import os as _os
_os.environ.setdefault("JAX_PLATFORMS", "cpu")
import jax
import jax.numpy as jnp

def _softmax(x, axis=-1):
    return jax.nn.softmax(x, axis=axis)
def _gelu(x):
    return jax.nn.gelu(x, approximate=True)
def _silu(x):
    return jax.nn.silu(x)
def _sigmoid(x):
    return jax.nn.sigmoid(x)
def _layernorm(x, axis=-1, eps=1e-5):
    m = jnp.mean(x, axis=axis, keepdims=True)
    v = jnp.var(x, axis=axis, keepdims=True)
    return (x - m) / jnp.sqrt(v + eps)
def _scatter_add(tgt, idx, src, axis=0):
    return tgt.at[idx].add(src)
def _segment_sum(src, seg, n):
    return jax.ops.segment_sum(src, seg, n)
class _Rng:
    def __init__(self, key):
        self._k = key
    def _next(self):
        self._k, sub = jax.random.split(self._k)
        return sub
    def normal(self, shape):
        return jax.random.normal(self._next(), shape, dtype=jnp.bfloat16)
    def randint(self, lo, hi, shape):
        return jax.random.randint(self._next(), shape, lo, hi, dtype=jnp.int32)
    def uniform(self, shape, lo=0.0, hi=1.0):
        return jax.random.uniform(self._next(), shape, jnp.bfloat16, lo, hi)
    def permutation(self, n):
        return jax.random.permutation(self._next(), n)


kernel_name = 'gated_mix__linear_kernel_hedgehog__glu_gated_bilinear__prompt'

def setup_inputs():
    _rng = _Rng(jax.random.key(int.from_bytes(__import__("os").urandom(4), "little")))
    _w = (lambda a: (lambda t: t.astype(jnp.bfloat16) if jnp.issubdtype(t.dtype, jnp.floating) else t)(jnp.asarray(a)))
    def _A_setup():
        B, S, D, H = 1, 2048, 512, 32
        Dh = D // H
        return {
            "x": _w((lambda *s: _rng.normal(s) * 0.05)(B, S, D)),
            "wqkv": _w((lambda *s: _rng.normal(s) * 0.8)(D, 3 * D)),
            "w_phi": _w((lambda *s: _rng.normal(s) * 0.8)(H, Dh, Dh) * (Dh ** -0.5)),
            "wo": _w((lambda *s: _rng.normal(s) * 0.05)(D, D)),
        }
    _A_in = _A_setup()

    def _B_setup():
        B, S, D, F = 1, 2048, 512, 1792
        return {
            "x": _w((lambda *s: _rng.normal(s) * 0.05)(B, S, D)),
            "w_gate": _w((lambda *s: _rng.normal(s) * 1.6)(D, F) * (D ** -0.5)),
            "w_up": _w((lambda *s: _rng.normal(s) * 1.6)(D, F) * (D ** -0.5)),
            "w_down": _w((lambda *s: _rng.normal(s) * 1.6)(F, D) * (F ** -0.5)),
        }
    _B_in = _B_setup()

    return {
        "A_x": _A_in["x"],
        "A_wqkv": _A_in["wqkv"],
        "A_w_phi": _A_in["w_phi"],
        "A_wo": _A_in["wo"],
        "B_x": _B_in["x"],
        "B_w_gate": _B_in["w_gate"],
        "B_w_up": _B_in["w_up"],
        "B_w_down": _B_in["w_down"],
        "gate_w": _w((lambda *s: _rng.normal(s) * 0.05)(512) * 16.0),
    }

def reference(A_x, A_wqkv, A_w_phi, A_wo, B_x, B_w_gate, B_w_up, B_w_down, gate_w):
    def _A_ref(x, wqkv, w_phi, wo):
        B, S, D = x.shape
        H = 32; Dh = D // H
        qkv = (lambda x, *d: x.transpose(*d))((x @ wqkv).reshape(B, S, 3, H, Dh), 2, 0, 3, 1, 4)
        q, k, v = qkv[0], qkv[1], qkv[2]
        pq = jnp.einsum("bhsd,hdf->bhsf", q, w_phi)
        pk = jnp.einsum("bhsd,hdf->bhsf", k, w_phi)
        phi_q = jnp.concatenate([_softmax(pq, axis=-1), _softmax(-pq, axis=-1)], axis=-1)
        phi_k = jnp.concatenate([_softmax(pk, axis=-1), _softmax(-pk, axis=-1)], axis=-1)
        kv = jnp.einsum("bhsf,bhsd->bhfd", phi_k, v)
        z  = jnp.einsum("bhsf->bhf", phi_k)
        num = jnp.einsum("bhqf,bhfd->bhqd", phi_q, kv)
        den = jnp.einsum("bhqf,bhf->bhq", phi_q, z)[..., None] + 1e-6
        o = num / den
        return (lambda x, *d: x.transpose(*d))(o, 0, 2, 1, 3).reshape(B, S, D) @ wo

    def _B_ref(x, w_gate, w_up, w_down):
        g = jnp.einsum("bsd,df->bsf", x, w_gate)
        u = jnp.einsum("bsd,df->bsf", x, w_up)
        h = g * u
        return jnp.einsum("bsf,fd->bsd", h, w_down)

    x = A_x
    g = _sigmoid((x * gate_w).sum(-1, keepdims=True))
    a = _A_ref(x, A_wqkv, A_w_phi, A_wo)
    b = _B_ref(x, B_w_gate, B_w_up, B_w_down)
    return g * a + (1 - g) * b
```

```python
import functools
import jax
import jax.numpy as jnp
from jax import lax
import jax.experimental.pallas as pl
import jax.experimental.pallas.tpu as pltpu

S, D, H, DH, F = 2048, 512, 32, 16, 1792
G = 4
HL = 8
TB = 512
NB = S // TB

f32 = jnp.float32
bf16 = jnp.bfloat16
NT = (((1,), (1,)), ((), ()))
NN = (((1,), (0,)), ((), ()))


def _dot(a, b, dims=NN):
    return lax.dot_general(a, b, dims, preferred_element_type=f32)


def _softmax_pair(p):
    t = p.shape[-1]
    p3 = p.reshape(DH, HL, t)
    mx = jnp.max(p3, axis=0, keepdims=True)
    mn = jnp.min(p3, axis=0, keepdims=True)
    ep = jnp.exp(p3 - mx)
    en = jnp.exp(mn - p3)
    zp = jnp.sum(ep, axis=0, keepdims=True)
    zn = jnp.sum(en, axis=0, keepdims=True)
    return ep, en, 1.0 / zp, 1.0 / zn


def kernel(x_ref, wqkv_ref, wphi_ref, wo_ref, wg_ref, wu_ref, wd_ref, gw_ref,
           o_ref, wqt_ref, wkt_ref, kv_ref, z_ref, kvt_ref, zb_ref, h_ref):
    phase = pl.program_id(0)
    i = pl.program_id(1)

    @pl.when((phase == 0) & (i == 0))
    def _prep():
        r = lax.broadcasted_iota(jnp.int32, (128, DH), 0)
        c = lax.broadcasted_iota(jnp.int32, (128, DH), 1)
        et = jnp.where((r // HL) == c, 1.0, 0.0).astype(bf16)
        rr = lax.broadcasted_iota(jnp.int32, (128, 128), 0)
        cc = lax.broadcasted_iota(jnp.int32, (128, 128), 1)
        mask = (rr % HL) == (cc // DH)
        for j in range(G):
            w2 = wphi_ref[j * 128:(j + 1) * 128, :]
            bj = _dot(et, w2, NT)
            bj = jnp.where(mask, bj, 0.0).astype(bf16)
            wq = wqkv_ref[:, j * 128:(j + 1) * 128]
            wk = wqkv_ref[:, D + j * 128:D + (j + 1) * 128]
            wqt_ref[j * 128:(j + 1) * 128, :] = _dot(bj, wq, NT).astype(bf16)
            wkt_ref[j * 128:(j + 1) * 128, :] = _dot(bj, wk, NT).astype(bf16)
        kv_ref[...] = jnp.zeros_like(kv_ref)
        z_ref[...] = jnp.zeros_like(z_ref)

    row0 = pl.multiple_of(i * TB, TB)

    @pl.when(phase == 0)
    def _phase0():
        x = x_ref[pl.ds(row0, TB), :]
        pk = _dot(wkt_ref[...], x, NT)
        v = _dot(x, wqkv_ref[:, 2 * D:3 * D]).astype(bf16)
        for j in range(G):
            ep, en, rp, rn = _softmax_pair(pk[j * 128:(j + 1) * 128, :])
            php = (ep * rp).reshape(128, TB)
            phn = (en * rn).reshape(128, TB)
            ph = jnp.concatenate([php, phn], axis=0)
            zs = ph[:, 0:128]
            for c in range(1, TB // 128):
                zs = zs + ph[:, c * 128:(c + 1) * 128]
            z_ref[j] += zs
            kv_ref[j] += _dot(ph.astype(bf16), v[:, j * 128:(j + 1) * 128])
        g = _dot(x, wg_ref[...])
        u = _dot(x, wu_ref[...])
        h_ref[pl.ds(row0, TB), :] = (g * u).astype(bf16)

    @pl.when((phase == 1) & (i == 0))
    def _mid():
        rr = lax.broadcasted_iota(jnp.int32, (128, 256), 0)
        cc = lax.broadcasted_iota(jnp.int32, (128, 256), 1)
        mask = (rr // DH) == (cc % HL)
        for j in range(G):
            kvt = kv_ref[j].T
            kvt_ref[j] = jnp.where(mask, kvt, 0.0).astype(bf16)
            zb_ref[j] = jnp.broadcast_to(jnp.sum(z_ref[j], axis=1, keepdims=True), (256, 128))

    @pl.when(phase == 1)
    def _phase1():
        x = x_ref[pl.ds(row0, TB), :]
        pq = _dot(wqt_ref[...], x, NT)
        ots = []
        for j in range(G):
            ep, en, rp, rn = _softmax_pair(pq[j * 128:(j + 1) * 128, :])
            zb = zb_ref[j]
            zbt = jnp.concatenate([zb] * (TB // 128), axis=1)
            zp = zbt[0:128].reshape(DH, HL, TB)
            zn = zbt[128:256].reshape(DH, HL, TB)
            dp = jnp.sum(ep * zp, axis=0, keepdims=True)
            dn = jnp.sum(en * zn, axis=0, keepdims=True)
            den = dp * rp + dn * rn + 1e-6
            rd = 1.0 / den
            php = (ep * (rp * rd)).reshape(128, TB)
            phn = (en * (rn * rd)).reshape(128, TB)
            ph = jnp.concatenate([php, phn], axis=0).astype(bf16)
            ot = _dot(kvt_ref[j], ph)
            ots.append(ot.T.astype(bf16))
        o = jnp.concatenate(ots, axis=1)
        a = _dot(o, wo_ref[...])
        b = _dot(h_ref[pl.ds(row0, TB), :], wd_ref[...])
        gl = jnp.sum(x.astype(f32) * gw_ref[...].astype(f32), axis=1, keepdims=True)
        g = jax.nn.sigmoid(gl)
        o_ref[...] = (g * a + (1.0 - g) * b).astype(o_ref.dtype)


@jax.jit
def pallas_gated_mix__linear_kernel_hedgehog__glu_gated_bilinear__prompt_kernel(
    A_x, A_wqkv, A_w_phi, A_wo, B_x, B_w_gate, B_w_up, B_w_down, gate_w,
):
    x = A_x.reshape(S, D)
    wphi = A_w_phi.reshape(H * DH, DH)
    gw = gate_w.reshape(1, D)

    def full(shape):
        return pl.BlockSpec(shape, lambda p, i: (0,) * len(shape))

    out = pl.pallas_call(
        kernel,
        grid=(2, NB),
        in_specs=[full((S, D)), full((D, 3 * D)), full((H * DH, DH)), full((D, D)),
                  full((D, F)), full((D, F)), full((F, D)), full((1, D))],
        out_specs=pl.BlockSpec((TB, D), lambda p, i: (i * p, 0)),
        out_shape=jax.ShapeDtypeStruct((S, D), A_x.dtype),
        scratch_shapes=[
            pltpu.VMEM((D, D), bf16),
            pltpu.VMEM((D, D), bf16),
            pltpu.VMEM((G, 256, 128), f32),
            pltpu.VMEM((G, 256, 128), f32),
            pltpu.VMEM((G, 128, 256), bf16),
            pltpu.VMEM((G, 256, 128), f32),
            pltpu.VMEM((S, F), bf16),
        ],
        compiler_params=pltpu.CompilerParams(
            dimension_semantics=("arbitrary", "arbitrary"),
            vmem_limit_bytes=100 * 1024 * 1024,
        ),
    )(x, A_wqkv, wphi, A_wo, B_w_gate, B_w_up, B_w_down, gw)
    return out.reshape(1, S, D)
```

```python
import jax
import jax.numpy as jnp
from jax import lax
import jax.experimental.pallas as pl
import jax.experimental.pallas.tpu as pltpu

S, D, H, DH, F = 2048, 512, 32, 16, 1792
NG = 8
T = 512
NB = S // T
TH = T // 2
KH = D // 2
FH = F // 2
LAG = 1
OPIECES = ((0, TH), (TH, 128), (TH + 128, 128))
LOG2E = 1.4426950408889634

f32 = jnp.float32
bf16 = jnp.bfloat16
u32 = jnp.uint32
NT = (((1,), (1,)), ((), ()))
NN = (((1,), (0,)), ((), ()))


def _dot(a, b, dims=NN):
    return lax.dot_general(a, b, dims, preferred_element_type=f32)


def _pack(a):
    return pltpu.bitcast(a, u32)


def _unpack(a):
    return pltpu.bitcast(a, bf16)


def _recip(z):
    r = pl.reciprocal(z, approx=True)
    return r * (2.0 - z * r)


def _fold(op, r):
    return op(r, pltpu.roll(r, 4, 0))


def _softmax_pair(p):
    t = p.shape[-1]
    p3 = p.reshape(8, 8, t)
    mx = _fold(jnp.maximum, jnp.max(p3, axis=0))
    mn = _fold(jnp.minimum, jnp.min(p3, axis=0))
    ep = jnp.exp2(p3 - mx[None])
    en = jnp.exp2(mn[None] - p3)
    zp = _fold(jnp.add, jnp.sum(ep, axis=0))
    zn = _fold(jnp.add, jnp.sum(en, axis=0))
    return ep, en, _recip(zp), _recip(zn)


LOPS = ((0, 3, 1), (2, 3, 1), (0, None, 0), (3, None, 0), (0, 1, 1), (2, 0, -1), (1, 3, -1))
ROPS = ((0, 3, 1), (0, None, 0), (1, 3, -1), (2, 0, -1), (3, None, 0), (0, 1, 1), (2, 3, 1))


def _ops7(table, q):
    return [q[a] if b is None else (q[a] + q[b] if s > 0 else q[a] - q[b]) for a, b, s in table]


def _op_from_bf16(table, k, q):
    a, b, s = table[k]
    if b is None:
        return q(a)
    fa, fb = q(a).astype(f32), q(b).astype(f32)
    return (fa + fb if s > 0 else fa - fb).astype(bf16)


def _c11(m):
    return m[0] + m[3] - m[4] + m[6]


def _c12(m):
    return m[2] + m[4]


def _c21(m):
    return m[1] + m[3]


def _c22(m):
    return m[0] - m[1] + m[2] + m[5]


ORDER = (2, 4, 1, 3, 0, 6, 5)
CQ = (_c12, _c21, _c11, _c22)
STEPS = ((2, 4), (1, 3), (0, 6), (5,))
QORDER = ((1, 0), (0, 1), (0, 0), (1, 1))


def _prep_t(dst_ref, lhs, w_ref, off=None, scale=None, js=(0, 1)):
    for j in js:
        if len(w_ref.shape) == 3:
            wt, wb = w_ref[j, :, 0:128], w_ref[j, :, 128:256]
        else:
            wt, wb = w_ref[:, 2 * j * 128:(2 * j + 1) * 128], w_ref[:, (2 * j + 1) * 128:(2 * j + 2) * 128]
        top = _dot(lhs[2 * j], wt, NT)
        bot = _dot(lhs[2 * j + 1], wb, NT)
        if scale is not None:
            top, bot = top * scale, bot * scale
        quads = [top[:, 0:KH], bot[:, 0:KH], top[:, KH:D], bot[:, KH:D]]
        for k, s in enumerate(_ops7(ROPS, quads)):
            s = _pack(s.astype(bf16))
            if off is None:
                dst_ref[k, j * 64:(j + 1) * 64, :] = s
            else:
                for t in range(2):
                    r0 = (2 * j + t) * 64 + off // 2
                    dst_ref[k, r0:r0 + 32, :] = s[t * 32:(t + 1) * 32, :]


def kernel(x_hbm, wqkv_hbm, wphi_hbm, wo_hbm, wg_hbm, wu_hbm, wd_hbm, gw_hbm,
           o_hbm,
           wphi_ref, gw_ref, x_ref, wq_ref, wk_ref, wv_ref, wo_ref, wg_ref, wu_ref, wd_ref, out_ref,
           wqt_ref, skv_ref, kvt_ref, zb_ref, sx_ref, sgu_ref, sd_ref, so_ref,
           xsem, wsem, osem, kvsem):
    def xcopy(i):
        return pltpu.make_async_copy(x_hbm.at[pl.ds(i * T, T), :], x_ref.at[pl.ds(i * T, T), :], xsem.at[i])

    def ocopy(i, p):
        r0, n = OPIECES[p]
        r = i * T + r0
        if not isinstance(i, int):
            r = pl.multiple_of(r, 64)
        return pltpu.make_async_copy(out_ref.at[pl.ds(r, n), :], o_hbm.at[pl.ds(r, n), :],
                                     osem.at[len(OPIECES) * i + p])

    def wkv_copy(j):
        return [pltpu.make_async_copy(wqkv_hbm.at[:, pl.ds(base + j * KH, KH)], dst.at[j],
                                      kvsem.at[n * 2 + j])
                for n, (base, dst) in enumerate(((D, wk_ref), (2 * D, wv_ref)))]

    c_wq = pltpu.make_async_copy(wqkv_hbm.at[:, pl.ds(0, D)], wq_ref, wsem.at[2])
    c_wg = pltpu.make_async_copy(wg_hbm, wg_ref, wsem.at[3])
    c_wu = pltpu.make_async_copy(wu_hbm, wu_ref, wsem.at[4])
    c_wd = pltpu.make_async_copy(wd_hbm, wd_ref, wsem.at[5])
    c_wo = pltpu.make_async_copy(wo_hbm, wo_ref, wsem.at[6])
    c_wphi = pltpu.make_async_copy(wphi_hbm, wphi_ref, wsem.at[7])
    c_gw = pltpu.make_async_copy(gw_hbm, gw_ref, wsem.at[8])

    c_wphi.start()
    for cp in wkv_copy(0):
        cp.start(priority=1)
    xcopy(0).start(priority=1)

    r = lax.broadcasted_iota(jnp.int32, (H, D), 0)
    c = lax.broadcasted_iota(jnp.int32, (H, D), 1)
    sel = jnp.where(r == c // DH, 1.0, 0.0).astype(bf16)
    r = lax.broadcasted_iota(jnp.int32, (256, D), 0)
    c = lax.broadcasted_iota(jnp.int32, (256, D), 1)
    m1 = (r // DH) == (c % DH)
    r = lax.broadcasted_iota(jnp.int32, (128, 256), 0)
    c = lax.broadcasted_iota(jnp.int32, (128, 256), 1)
    rsel = jnp.where(((r % 64) // 4) == (c % DH), 1.0, 0.0).astype(bf16)
    r = lax.broadcasted_iota(jnp.int32, (128, D), 0)
    c = lax.broadcasted_iota(jnp.int32, (128, D), 1)
    m2 = ((r // 64) * 4 + r % 4) == ((c // DH) % 8)
    r = lax.broadcasted_iota(jnp.int32, (128, 128), 0)
    c = lax.broadcasted_iota(jnp.int32, (128, 128), 1)
    eye = jnp.where(r == c, 1.0, 0.0).astype(bf16)

    c_wphi.wait()
    for cp in wkv_copy(1):
        cp.start(priority=1)
    xcopy(1).start(priority=1)
    t1 = _dot(wphi_ref[...], sel)
    t1 = jnp.where(m1, t1, 0.0).astype(bf16)
    ball = _dot(rsel, t1)
    ball = jnp.where(m2, ball, 0.0).astype(bf16)
    bjs = [ball[:, j * 128:(j + 1) * 128] for j in range(4)]

    def prep_kv(j):
        _prep_t(skv_ref, bjs, wk_ref, off=0, scale=LOG2E, js=(j,))
        _prep_t(skv_ref, [eye] * 4, wv_ref, off=64, js=(j,))

    for cp in wkv_copy(0):
        cp.wait()
    prep_kv(0)

    kv = [None] * NG
    zacc = [None] * NG

    def acc(lst, g, v):
        lst[g] = v if lst[g] is None else lst[g] + v

    def x_op(i, k, first):
        if not first:
            return _unpack(sx_ref[i, k])

        def q(n):
            r0 = i * T + (n // 2) * TH
            return x_ref[r0:r0 + TH, (n % 2) * KH:(n % 2 + 1) * KH]
        s = _op_from_bf16(LOPS, k, q)
        sx_ref[i, k] = _pack(s)
        return s

    def k_softmax(p, g):
        ep, en, rp, rn = _softmax_pair(p)
        ph = jnp.concatenate([(ep * rp[None]).reshape(64, TH), (en * rn[None]).reshape(64, TH)], axis=0)
        zs = ph[:, 0:128]
        for c in range(1, TH // 128):
            zs = zs + ph[:, c * 128:(c + 1) * 128]
        acc(zacc, g, zs)
        return ph.astype(bf16)

    def kv_group(q, gl, m):
        rh, half = QORDER[q]
        g = rh * 4 + gl
        c = CQ[q](m)
        acc(kv, g, _dot(c[64:128, :].astype(bf16), k_softmax(c[0:64, :], g), NT))

    pending = []

    def drain(n):
        for _ in range(min(n, len(pending))):
            kv_group(*pending.pop(0))

    rr = lax.broadcasted_iota(jnp.int32, (64, 128), 0)
    cc = lax.broadcasted_iota(jnp.int32, (64, 128), 1)
    mask2 = (rr // DH) == (cc % 4)

    def rhs_op(first, k, s_ref, quads, rows, cols):
        if not first:
            return _unpack(s_ref[k])

        def q(n):
            ref, r0, c0 = quads[n]
            return ref[r0:r0 + rows, c0:c0 + cols]
        s = _op_from_bf16(ROPS, k, q)
        s_ref[k] = _pack(s)
        return s

    gu_q = ((wg_ref, 0, 0), (wu_ref, 0, 0), (wg_ref, KH, 0), (wu_ref, KH, 0))
    wd_q = ((wd_ref, 0, 0), (wd_ref, 0, KH), (wd_ref, FH, 0), (wd_ref, FH, KH))
    wo_q = ((wo_ref, 0, 0), (wo_ref, 0, KH), (wo_ref, KH, 0), (wo_ref, KH, KH))

    def phase_b(i, first, hook=None):
        row0 = i * T if first else pl.multiple_of(i * T, T)

        qm = [None] * 7
        for k in ORDER:
            qm[k] = _dot(_unpack(wqt_ref[k]), x_op(i, k, False), NT)
        if hook is not None:
            hook()

        gm = [None] * 7

        def gu(k):
            gm[k] = _dot(x_op(i, k, False), rhs_op(first, k, sgu_ref, gu_q, KH, F))

        gu(2)
        gu(4)
        u_top = _c12(gm)

        ot = {}
        for q, (rh, half) in enumerate(QORDER):
            pq = CQ[q](qm)
            for gl in range(4):
                g = rh * 4 + gl
                ep, en, rp, rn = _softmax_pair(pq[gl * 64:(gl + 1) * 64, :])
                zb = zb_ref[g]
                zbt = jnp.concatenate([zb] * (TH // 128), axis=1)
                dp = jnp.sum(ep * zbt[0:64].reshape(8, 8, TH), axis=0)
                dn = jnp.sum(en * zbt[64:128].reshape(8, 8, TH), axis=0)
                den = _fold(jnp.add, dp * rp + dn * rn) + 1e-6
                rd = 1.0 / den
                php = (ep * (rp * rd)[None]).reshape(64, TH)
                phn = (en * (rn * rd)[None]).reshape(64, TH)
                ph = jnp.concatenate([php, phn], axis=0).astype(bf16)
                ot[(g, half)] = _dot(_unpack(kvt_ref[g]), ph)

        def oq(half, ch):
            blocks = []
            for j in range(2):
                ob = 2 * ch + j
                b = (ob // 2) + 2 * (ob % 2)
                blocks.append(jnp.concatenate([ot[(2 * b, half)], ot[(2 * b + 1, half)]], axis=0).T)
            return jnp.concatenate(blocks, axis=1)

        gu(1)
        gu(3)
        g_bot = _c21(gm)
        gu(0)
        gu(6)
        h_top = _c11(gm) * u_top
        gu(5)
        h_bot = g_bot * _c22(gm)

        x = x_ref[pl.ds(row0, T), :]
        gwf = gw_ref[...].astype(f32)
        xg = x[:, 0:128].astype(f32) * gwf[0:1, :]
        for c in range(1, 4):
            xg = xg + x[:, c * 128:(c + 1) * 128].astype(f32) * gwf[c:c + 1, :]
        gate = jax.nn.sigmoid(jnp.sum(xg, axis=1, keepdims=True))
        g_t, g_b = gate[0:TH], gate[TH:T]

        ol = [t.astype(bf16) for t in _ops7(LOPS, [oq(0, 0), oq(0, 1), oq(1, 0), oq(1, 1)])]
        am = [None] * 7
        for k in ORDER:
            am[k] = _dot(ol[k], rhs_op(first, k, so_ref, wo_q, KH, KH))

        hl = [t.astype(bf16) for t in _ops7(LOPS, [h_top[:, 0:FH], h_top[:, FH:F], h_bot[:, 0:FH], h_bot[:, FH:F]])]
        bm = [None] * 7

        def down(k):
            bm[k] = _dot(hl[k], rhs_op(first, k, sd_ref, wd_q, FH, KH))

        def emit(cf, gq, r0, c0):
            out_ref[pl.ds(row0 + r0, TH), c0:c0 + KH] = (gq * cf(am) + (1.0 - gq) * cf(bm)).astype(out_ref.dtype)

        down(2)
        down(4)
        emit(_c12, g_t, 0, KH)
        down(3)
        down(0)
        down(6)
        emit(_c11, g_t, 0, 0)
        ocopy(i, 0).start()
        down(1)
        emit(_c21, g_b, TH, 0)
        r5 = rhs_op(first, 5, sd_ref, wd_q, FH, KH)
        for p in range(1, len(OPIECES)):
            r0, n = OPIECES[p][0] - TH, OPIECES[p][1]
            rows = slice(r0, r0 + n)
            bp = [None if m is None else m[rows] for m in bm]
            bp[5] = _dot(hl[5][rows], r5)
            res = g_b[rows] * _c22([m[rows] for m in am]) + (1.0 - g_b[rows]) * _c22(bp)
            out_ref[pl.ds(row0 + TH + r0, n), KH:D] = res.astype(out_ref.dtype)
            ocopy(i, p).start()

    xcopy(0).wait()
    for cp in (xcopy(2), xcopy(3), c_wq, c_wg, c_wu, c_wd, c_wo, c_gw):
        cp.start(priority=1)
    for i in range(NB):
        for gl in range(4):
            if (i, gl) == (0, 2):
                for cp in wkv_copy(1):
                    cp.wait()
                xcopy(1).wait()
                prep_kv(1)
            if (i, gl) == (2, 0):
                xcopy(2).wait()
                xcopy(3).wait()
            m = [None] * 7
            for q in range(4):
                for k in STEPS[q]:
                    m[k] = _dot(_unpack(skv_ref[k, gl * 64:(gl + 1) * 64, :]), x_op(i, k, gl == 0), NT)
                drain(len(pending) - LAG)
                pending.append((q, gl, list(m)))
    c_wg.wait()
    c_wu.wait()
    c_wd.wait()
    c_wq.wait()
    c_wo.wait()
    c_gw.wait()
    _prep_t(wqt_ref, bjs, wq_ref, scale=LOG2E)

    def finish_a():
        drain(len(pending))
        for g in range(NG):
            kvt_ref[g] = _pack(jnp.where(mask2, kv[g], 0.0).astype(bf16))
            zb_ref[g] = jnp.broadcast_to(jnp.sum(zacc[g], axis=1, keepdims=True), (128, 128))

    phase_b(0, True, finish_a)

    def body(i, carry):
        phase_b(i, False)
        return carry

    lax.fori_loop(1, NB, body, 0)
    for i in range(NB):
        for p in range(len(OPIECES)):
            ocopy(i, p).wait()


@jax.jit
def pallas_gated_mix__linear_kernel_hedgehog__glu_gated_bilinear__prompt_kernel(
    A_x, A_wqkv, A_w_phi, A_wo, B_x, B_w_gate, B_w_up, B_w_down, gate_w,
):
    x = A_x.reshape(S, D)
    wphi = jnp.transpose(A_w_phi, (1, 2, 0)).reshape(DH * DH, H)
    gw = gate_w.reshape(4, 128)

    hbm = pl.BlockSpec(memory_space=pl.ANY)

    out = pl.pallas_call(
        kernel,
        in_specs=[hbm] * 8,
        out_specs=hbm,
        out_shape=jax.ShapeDtypeStruct((S, D), A_x.dtype),
        scratch_shapes=[
            pltpu.VMEM((DH * DH, H), bf16),
            pltpu.VMEM((4, 128), bf16),
            pltpu.VMEM((S, D), bf16),
            pltpu.VMEM((D, D), bf16),
            pltpu.VMEM((2, D, KH), bf16),
            pltpu.VMEM((2, D, KH), bf16),
            pltpu.VMEM((D, D), bf16),
            pltpu.VMEM((D, F), bf16),
            pltpu.VMEM((D, F), bf16),
            pltpu.VMEM((F, D), bf16),
            pltpu.VMEM((S, D), bf16),
            pltpu.VMEM((7, KH // 2, KH), u32),
            pltpu.VMEM((7, D // 2, KH), u32),
            pltpu.VMEM((NG, 32, 128), u32),
            pltpu.VMEM((NG, 128, 128), f32),
            pltpu.VMEM((NB, 7, TH // 2, KH), u32),
            pltpu.VMEM((7, KH // 2, F), u32),
            pltpu.VMEM((7, FH // 2, KH), u32),
            pltpu.VMEM((7, KH // 2, KH), u32),
            pltpu.SemaphoreType.DMA((NB,)),
            pltpu.SemaphoreType.DMA((9,)),
            pltpu.SemaphoreType.DMA((len(OPIECES) * NB,)),
            pltpu.SemaphoreType.DMA((4,)),
        ],
        compiler_params=pltpu.CompilerParams(
            vmem_limit_bytes=100 * 1024 * 1024,
        ),
    )(x, A_wqkv, wphi, A_wo, B_w_gate, B_w_up, B_w_down, gw)
    return out.reshape(1, S, D)
```

```python
import jax
import jax.numpy as jnp
from jax import lax
import jax.experimental.pallas as pl
import jax.experimental.pallas.tpu as pltpu

S, D, H, DH, F = 2048, 512, 32, 16, 1792
NG = 8
T = 512
NB = S // T
TH = T // 2
KH = D // 2
FH = F // 2
LAG = 3
QC0 = 1
LATE_FIRST = False
LATE_LOOP = False
QN0 = 2
OPIECES = ((0, TH), (TH, 128), (TH + 128, 128))
LOG2E = 1.4426950408889634

f32 = jnp.float32
bf16 = jnp.bfloat16
u32 = jnp.uint32
NT = (((1,), (1,)), ((), ()))
NN = (((1,), (0,)), ((), ()))


def _dot(a, b, dims=NN):
    return lax.dot_general(a, b, dims, preferred_element_type=f32)


def _pack(a):
    return pltpu.bitcast(a, u32)


def _unpack(a):
    return pltpu.bitcast(a, bf16)


def _lin(a, b, s):
    return a + b if s > 0 else a - b


def _ops2(table, k1, blk):
    a, b, s = table[k1]
    sub = []
    for n2 in range(4):
        v = blk(a, n2).astype(f32)
        if b is not None:
            v = _lin(v, blk(b, n2).astype(f32), s)
        sub.append(v)
    out = []
    for a2, b2, s2 in table:
        if b is None and b2 is None:
            out.append(_pack(blk(a, a2)))
        else:
            out.append(_pack((sub[a2] if b2 is None else _lin(sub[a2], sub[b2], s2)).astype(bf16)))
    return out


def _recip(z):
    r = pl.reciprocal(z, approx=True)
    return r * (2.0 - z * r)


def _fold(op, r):
    return op(r, pltpu.roll(r, 4, 0))


def _softmax_pair(p):
    t = p.shape[-1]
    p3 = p.reshape(8, 8, t)
    mx = _fold(jnp.maximum, jnp.max(p3, axis=0))
    mn = _fold(jnp.minimum, jnp.min(p3, axis=0))
    ep = jnp.exp2(p3 - mx[None])
    en = jnp.exp2(mn[None] - p3)
    zp = _fold(jnp.add, jnp.sum(ep, axis=0))
    zn = _fold(jnp.add, jnp.sum(en, axis=0))
    return ep, en, _recip(zp), _recip(zn)


LOPS = ((0, 3, 1), (2, 3, 1), (0, None, 0), (3, None, 0), (0, 1, 1), (2, 0, -1), (1, 3, -1))
ROPS = ((0, 3, 1), (0, None, 0), (1, 3, -1), (2, 0, -1), (3, None, 0), (0, 1, 1), (2, 3, 1))


def _ops7(table, q):
    return [q[a] if b is None else (q[a] + q[b] if s > 0 else q[a] - q[b]) for a, b, s in table]


def _op_from_bf16(table, k, q):
    a, b, s = table[k]
    if b is None:
        return q(a)
    fa, fb = q(a).astype(f32), q(b).astype(f32)
    return (fa + fb if s > 0 else fa - fb).astype(bf16)


def _c11(m):
    return ((m[3] - m[4]) + m[0]) + m[6]


def _c12(m):
    return m[2] + m[4]


def _c21(m):
    return m[1] + m[3]


def _c22(m):
    return ((m[2] - m[1]) + m[0]) + m[5]


def _c11_lazy(m):
    return ((m[6] + m[0]) + m[3]) - m[4]


def _c22_lazy(m):
    return ((m[5] + m[0]) + m[2]) - m[1]


ORDER = (2, 4, 1, 3, 0, 6, 5)
CQ = (_c12, _c21, _c11, _c22)
STEPS = ((2, 4), (1, 3), (0, 6), (5,))
QORDER = ((1, 0), (0, 1), (0, 0), (1, 1))


def _prep_t(dst_ref, lhs, w_ref, off=None, scale=None, js=(0, 1)):
    for j in js:
        if len(w_ref.shape) == 3:
            wt, wb = w_ref[j, :, 0:128], w_ref[j, :, 128:256]
        else:
            wt, wb = w_ref[:, 2 * j * 128:(2 * j + 1) * 128], w_ref[:, (2 * j + 1) * 128:(2 * j + 2) * 128]
        top = _dot(lhs[2 * j], wt, NT)
        bot = _dot(lhs[2 * j + 1], wb, NT)
        if scale is not None:
            top, bot = top * scale, bot * scale
        quads = [top[:, 0:KH], bot[:, 0:KH], top[:, KH:D], bot[:, KH:D]]
        for k, s in enumerate(_ops7(ROPS, quads)):
            s = _pack(s.astype(bf16))
            if off is None:
                dst_ref[k, j * 64:(j + 1) * 64, :] = s
            else:
                for t in range(2):
                    r0 = (2 * j + t) * 64 + off // 2
                    dst_ref[k, r0:r0 + 32, :] = s[t * 32:(t + 1) * 32, :]


def kernel(x_hbm, wqkv_hbm, wphi_hbm, wo_hbm, wg_hbm, wu_hbm, wd_hbm, gw_hbm,
           o_hbm,
           wphi_ref, gw_ref, x_ref, wq_ref, wk_ref, wv_ref, wo_ref, wg_ref, wu_ref, wd_ref, out_ref,
           wqt_ref, skv_ref, kvt_ref, zb_ref, sx_ref, sx2_ref, sgu_ref, sd_ref, so_ref,
           xsem, wsem, osem, kvsem):
    def xcopy(i):
        return pltpu.make_async_copy(x_hbm.at[pl.ds(i * T, T), :], x_ref.at[pl.ds(i * T, T), :], xsem.at[i])

    def ocopy(i, p):
        r0, n = OPIECES[p]
        r = i * T + r0
        if not isinstance(i, int):
            r = pl.multiple_of(r, 64)
        return pltpu.make_async_copy(out_ref.at[pl.ds(r, n), :], o_hbm.at[pl.ds(r, n), :],
                                     osem.at[len(OPIECES) * i + p])

    def wkv_copy(j):
        return [pltpu.make_async_copy(wqkv_hbm.at[:, pl.ds(base + j * KH, KH)], dst.at[j],
                                      kvsem.at[n * 2 + j])
                for n, (base, dst) in enumerate(((D, wk_ref), (2 * D, wv_ref)))]

    c_wq = pltpu.make_async_copy(wqkv_hbm.at[:, pl.ds(0, D)], wq_ref, wsem.at[2])
    c_wg = pltpu.make_async_copy(wg_hbm, wg_ref, wsem.at[3])
    c_wu = pltpu.make_async_copy(wu_hbm, wu_ref, wsem.at[4])
    c_wd = pltpu.make_async_copy(wd_hbm, wd_ref, wsem.at[5])
    c_wo = pltpu.make_async_copy(wo_hbm, wo_ref, wsem.at[6])
    c_wphi = pltpu.make_async_copy(wphi_hbm, wphi_ref, wsem.at[7])
    c_gw = pltpu.make_async_copy(gw_hbm, gw_ref, wsem.at[8])

    c_wphi.start()
    for cp in wkv_copy(0):
        cp.start(priority=1)
    xcopy(0).start(priority=1)

    r = lax.broadcasted_iota(jnp.int32, (H, D), 0)
    c = lax.broadcasted_iota(jnp.int32, (H, D), 1)
    sel = jnp.where(r == c // DH, 1.0, 0.0).astype(bf16)
    r = lax.broadcasted_iota(jnp.int32, (256, D), 0)
    c = lax.broadcasted_iota(jnp.int32, (256, D), 1)
    m1 = (r // DH) == (c % DH)
    r = lax.broadcasted_iota(jnp.int32, (128, 256), 0)
    c = lax.broadcasted_iota(jnp.int32, (128, 256), 1)
    rsel = jnp.where(((r % 64) // 4) == (c % DH), 1.0, 0.0).astype(bf16)
    r = lax.broadcasted_iota(jnp.int32, (128, D), 0)
    c = lax.broadcasted_iota(jnp.int32, (128, D), 1)
    m2 = ((r // 64) * 4 + r % 4) == ((c // DH) % 8)
    r = lax.broadcasted_iota(jnp.int32, (128, 128), 0)
    c = lax.broadcasted_iota(jnp.int32, (128, 128), 1)
    eye = jnp.where(r == c, 1.0, 0.0).astype(bf16)

    c_wphi.wait()
    for cp in wkv_copy(1):
        cp.start(priority=1)
    xcopy(1).start(priority=1)
    t1 = _dot(wphi_ref[...], sel)
    t1 = jnp.where(m1, t1, 0.0).astype(bf16)
    ball = _dot(rsel, t1)
    ball = jnp.where(m2, ball, 0.0).astype(bf16)
    bjs = [ball[:, j * 128:(j + 1) * 128] for j in range(4)]

    def prep_kv(j):
        _prep_t(skv_ref, bjs, wk_ref, off=0, scale=LOG2E, js=(j,))
        _prep_t(skv_ref, [eye] * 4, wv_ref, off=64, js=(j,))

    for cp in wkv_copy(0):
        cp.wait()
    prep_kv(0)

    kv = [None] * NG
    zacc = [None] * NG

    def acc(lst, g, v):
        lst[g] = v if lst[g] is None else lst[g] + v

    def x_op(i, k, first):
        if not first:
            return _unpack(sx_ref[i, k])

        def q(n):
            r0 = i * T + (n // 2) * TH
            return x_ref[r0:r0 + TH, (n % 2) * KH:(n % 2 + 1) * KH]
        s = _op_from_bf16(LOPS, k, q)
        sx_ref[i, k] = _pack(s)
        return s

    def kv_group(q, gl, ch, m):
        rh, half = QORDER[q]
        g = rh * 4 + gl
        c = CQ[q]([None if t is None else t[:, ch * 128:(ch + 1) * 128] for t in m])
        ep, en, rp, rn = _softmax_pair(c[0:64, :])
        ph = jnp.concatenate([(ep * rp[None]).reshape(64, 128), (en * rn[None]).reshape(64, 128)], axis=0)
        acc(zacc, g, ph)
        acc(kv, g, _dot(c[64:128, :].astype(bf16), ph.astype(bf16), NT))

    pending = []

    def drain(n):
        for _ in range(min(n, len(pending))):
            kv_group(*pending.pop(0))

    rr = lax.broadcasted_iota(jnp.int32, (64, 128), 0)
    cc = lax.broadcasted_iota(jnp.int32, (64, 128), 1)
    mask2 = (rr // DH) == (cc % 4)

    def rhs_op(first, k, s_ref, quads, rows, cols):
        if not first:
            return _unpack(s_ref[k])

        def q(n):
            ref, r0, c0 = quads[n]
            return ref[r0:r0 + rows, c0:c0 + cols]
        s = _op_from_bf16(ROPS, k, q)
        s_ref[k] = _pack(s)
        return s

    gu_q = ((wg_ref, 0, 0), (wu_ref, 0, 0), (wg_ref, KH, 0), (wu_ref, KH, 0))
    wd_q = ((wd_ref, 0, 0), (wd_ref, 0, KH), (wd_ref, FH, 0), (wd_ref, FH, KH))
    wo_q = ((wo_ref, 0, 0), (wo_ref, 0, KH), (wo_ref, KH, 0), (wo_ref, KH, KH))

    def phase_b(i, first, hook=None):
        row0 = i * T if first else pl.multiple_of(i * T, T)
        late = LATE_FIRST if first else LATE_LOOP

        qm = [None] * 7
        ot = {}

        def pq_prod(k):
            qm[k] = _dot(_unpack(wqt_ref[k]), x_op(i, k, False), NT)

        qs = {}

        def pq_slice(k, gl):
            qs[(k, gl)] = _dot(_unpack(wqt_ref[k, gl * 32:(gl + 1) * 32, :]), x_op(i, k, False), NT)

        def q_group(q, gl):
            rh, half = QORDER[q]
            g = rh * 4 + gl
            p = CQ[q]([qs.get((k, gl)) if qm[k] is None else qm[k][gl * 64:(gl + 1) * 64, :] for k in range(7)])
            ep, en, rp, rn = _softmax_pair(p)
            zb = zb_ref[g]
            zbt = jnp.concatenate([zb] * (TH // 128), axis=1)
            dp = jnp.sum(ep * zbt[0:64].reshape(8, 8, TH), axis=0)
            dn = jnp.sum(en * zbt[64:128].reshape(8, 8, TH), axis=0)
            den = _fold(jnp.add, dp * rp + dn * rn) + 1e-6
            rd = 1.0 / den
            php = (ep * (rp * rd)[None]).reshape(64, TH)
            phn = (en * (rn * rd)[None]).reshape(64, TH)
            ph = jnp.concatenate([php, phn], axis=0).astype(bf16)
            ot[(g, half)] = _dot(_unpack(kvt_ref[g]), ph)

        def oq(half, ch):
            blocks = []
            for j in range(2):
                ob = 2 * ch + j
                b = (ob // 2) + 2 * (ob % 2)
                blocks.append(jnp.concatenate([ot[(2 * b, half)], ot[(2 * b + 1, half)]], axis=0).T)
            return jnp.concatenate(blocks, axis=1)

        for k in (2, 1, 0):
            pq_prod(k)
        if hook is not None:
            hook()

        TQ, FQ = T // 4, F // 2
        hc = [[None] * 14 for _ in range(4)]

        def xblk(n1, n2):
            r0 = (n1 // 2) * TH + (n2 // 2) * TQ
            c0 = (n1 % 2) * KH + (n2 % 2) * 128
            return x_ref[pl.ds(row0 + r0, TQ), c0:c0 + 128]

        for c in range(7):
            def wblk(n1, n2):
                ref = wu_ref if n1 % 2 else wg_ref
                r0 = (n1 // 2) * KH + (n2 // 2) * 128
                c0 = (n2 % 2) * FQ + c * 128
                return ref[r0:r0 + 128, c0:c0 + 128]
            q = -1 if late else c - QC0
            inner = [None] * 7
            for n, k1 in enumerate(ORDER):
                if 0 <= q < 4 and n < 4:
                    pq_slice(STEPS[q][-1], n)
                if c == 0:
                    for k2, t in enumerate(_ops2(LOPS, k1, xblk)):
                        sx2_ref[k1 * 7 + k2] = t
                if first:
                    for k2, t in enumerate(_ops2(ROPS, k1, wblk)):
                        sgu_ref[k1 * 7 + k2, :, c * 128:(c + 1) * 128] = t
                xo = [sx2_ref[k1 * 7 + k2] for k2 in range(7)]
                wo_ = [sgu_ref[k1 * 7 + k2, :, c * 128:(c + 1) * 128] for k2 in range(7)]
                m = [None] * 7
                for k2 in ORDER:
                    m[k2] = _dot(_unpack(xo[k2]), _unpack(wo_[k2]))
                inner[k1] = [_c11(m), _c12(m), _c21(m), _c22(m)]
                if 0 <= q < 4 and QN0 <= n < QN0 + 4:
                    q_group(q, n - QN0)
            for sq in range(4):
                mm = [inner[k1][sq] for k1 in range(7)]
                rh, ch = sq // 2, sq % 2
                hc[rh][ch * 7 + c] = _c11_lazy(mm) * _c12(mm)
                hc[2 + rh][ch * 7 + c] = _c21(mm) * _c22_lazy(mm)

        h_top = jnp.concatenate([jnp.concatenate(hc[0], axis=1), jnp.concatenate(hc[1], axis=1)], axis=0)
        h_bot = jnp.concatenate([jnp.concatenate(hc[2], axis=1), jnp.concatenate(hc[3], axis=1)], axis=0)

        x = x_ref[pl.ds(row0, T), :]
        gwf = gw_ref[...].astype(f32)
        xg = x[:, 0:128].astype(f32) * gwf[0:1, :]
        for c in range(1, 4):
            xg = xg + x[:, c * 128:(c + 1) * 128].astype(f32) * gwf[c:c + 1, :]
        gate = jax.nn.sigmoid(jnp.sum(xg, axis=1, keepdims=True))
        g_t, g_b = gate[0:TH], gate[TH:T]

        am = [None] * 7

        def wo_prods():
            ol = [t.astype(bf16) for t in _ops7(LOPS, [oq(0, 0), oq(0, 1), oq(1, 0), oq(1, 1)])]
            for k in ORDER:
                am[k] = _dot(ol[k], rhs_op(first, k, so_ref, wo_q, KH, KH))

        hl = [t.astype(bf16) for t in _ops7(LOPS, [h_top[:, 0:FH], h_top[:, FH:F], h_bot[:, 0:FH], h_bot[:, FH:F]])]
        bm = [None] * 7

        def down(k):
            bm[k] = _dot(hl[k], rhs_op(first, k, sd_ref, wd_q, FH, KH))

        def emit(cf, gq, r0, c0):
            out_ref[pl.ds(row0 + r0, TH), c0:c0 + KH] = (gq * cf(am) + (1.0 - gq) * cf(bm)).astype(out_ref.dtype)

        if late:
            for q, k in enumerate((2, 4, 3, 0)):
                pq_prod(STEPS[q][-1])
                down(k)
                for gl in range(4):
                    q_group(q, gl)
            down(6)
            wo_prods()
            emit(_c12, g_t, 0, KH)
        else:
            wo_prods()
            down(2)
            down(4)
            emit(_c12, g_t, 0, KH)
            down(3)
            down(0)
            down(6)
        emit(_c11, g_t, 0, 0)
        ocopy(i, 0).start()
        down(1)
        emit(_c21, g_b, TH, 0)
        r5 = rhs_op(first, 5, sd_ref, wd_q, FH, KH)
        for p in range(1, len(OPIECES)):
            r0, n = OPIECES[p][0] - TH, OPIECES[p][1]
            rows = slice(r0, r0 + n)
            bp = [None if m is None else m[rows] for m in bm]
            bp[5] = _dot(hl[5][rows], r5)
            res = g_b[rows] * _c22([m[rows] for m in am]) + (1.0 - g_b[rows]) * _c22(bp)
            out_ref[pl.ds(row0 + TH + r0, n), KH:D] = res.astype(out_ref.dtype)
            ocopy(i, p).start()

    xcopy(0).wait()
    for cp in (xcopy(2), xcopy(3), c_wq, c_wg, c_wu, c_wd, c_wo, c_gw):
        cp.start(priority=1)
    for i in range(NB):
        for gl in range(4):
            if (i, gl) == (0, 2):
                for cp in wkv_copy(1):
                    cp.wait()
                xcopy(1).wait()
                prep_kv(1)
            if (i, gl) == (2, 0):
                xcopy(2).wait()
                xcopy(3).wait()
            m = [None] * 7
            for q in range(4):
                for k in STEPS[q]:
                    m[k] = _dot(_unpack(skv_ref[k, gl * 64:(gl + 1) * 64, :]), x_op(i, k, gl == 0), NT)
                    drain(min(2 if len(pending) > LAG + 2 else 1, len(pending) - LAG))
                pending.extend((q, gl, ch, list(m)) for ch in range(TH // 128))
    c_wg.wait()
    c_wu.wait()
    c_wd.wait()
    c_wq.wait()
    c_wo.wait()
    c_gw.wait()
    _prep_t(wqt_ref, bjs, wq_ref, scale=LOG2E)

    def finish_a():
        drain(len(pending))
        for g in range(NG):
            kvt_ref[g] = _pack(jnp.where(mask2, kv[g], 0.0).astype(bf16))
            zb_ref[g] = jnp.broadcast_to(jnp.sum(zacc[g], axis=1, keepdims=True), (128, 128))

    phase_b(0, True, finish_a)

    def body(i, carry):
        phase_b(i, False)
        return carry

    lax.fori_loop(1, NB, body, 0)
    for i in range(NB):
        for p in range(len(OPIECES)):
            ocopy(i, p).wait()


@jax.jit
def pallas_gated_mix__linear_kernel_hedgehog__glu_gated_bilinear__prompt_kernel(
    A_x, A_wqkv, A_w_phi, A_wo, B_x, B_w_gate, B_w_up, B_w_down, gate_w,
):
    x = A_x.reshape(S, D)
    wphi = jnp.transpose(A_w_phi, (1, 2, 0)).reshape(DH * DH, H)
    gw = gate_w.reshape(4, 128)

    hbm = pl.BlockSpec(memory_space=pl.ANY)

    out = pl.pallas_call(
        kernel,
        in_specs=[hbm] * 8,
        out_specs=hbm,
        out_shape=jax.ShapeDtypeStruct((S, D), A_x.dtype),
        scratch_shapes=[
            pltpu.VMEM((DH * DH, H), bf16),
            pltpu.VMEM((4, 128), bf16),
            pltpu.VMEM((S, D), bf16),
            pltpu.VMEM((D, D), bf16),
            pltpu.VMEM((2, D, KH), bf16),
            pltpu.VMEM((2, D, KH), bf16),
            pltpu.VMEM((D, D), bf16),
            pltpu.VMEM((D, F), bf16),
            pltpu.VMEM((D, F), bf16),
            pltpu.VMEM((F, D), bf16),
            pltpu.VMEM((S, D), bf16),
            pltpu.VMEM((7, KH // 2, KH), u32),
            pltpu.VMEM((7, D // 2, KH), u32),
            pltpu.VMEM((NG, 32, 128), u32),
            pltpu.VMEM((NG, 128, 128), f32),
            pltpu.VMEM((NB, 7, TH // 2, KH), u32),
            pltpu.VMEM((49, T // 8, 128), u32),
            pltpu.VMEM((49, 64, F // 2), u32),
            pltpu.VMEM((7, FH // 2, KH), u32),
            pltpu.VMEM((7, KH // 2, KH), u32),
            pltpu.SemaphoreType.DMA((NB,)),
            pltpu.SemaphoreType.DMA((9,)),
            pltpu.SemaphoreType.DMA((len(OPIECES) * NB,)),
            pltpu.SemaphoreType.DMA((4,)),
        ],
        compiler_params=pltpu.CompilerParams(
            vmem_limit_bytes=100 * 1024 * 1024,
        ),
    )(x, A_wqkv, wphi, A_wo, B_w_gate, B_w_up, B_w_down, gw)
    return out.reshape(1, S, D)
```

```python
import jax
import jax.numpy as jnp
from jax import lax
import jax.experimental.pallas as pl
import jax.experimental.pallas.tpu as pltpu

S, D, H, DH, F = 2048, 512, 32, 16, 1792
NG = 8
T = 512
NB = S // T
TH, TQ = T // 2, T // 4
KH, FH = D // 2, F // 2
LAG = 3
P0, PLAG = 14, 2
OPIECES = ((0, TH), (TH, 128), (TH + 128, 128))
LOG2E = 1.4426950408889634

f32 = jnp.float32
bf16 = jnp.bfloat16
NT = (((1,), (1,)), ((), ()))
NN = (((1,), (0,)), ((), ()))


def _dot(a, b, dims=NN):
    return lax.dot_general(a, b, dims, preferred_element_type=f32)


def _recip(z):
    r = pl.reciprocal(z, approx=True)
    return r * (2.0 - z * r)


def _fold(op, r):
    return op(r, pltpu.roll(r, 4, 0))


def _softmax_pair(p):
    p3 = p.reshape(8, 8, p.shape[-1])
    mx = _fold(jnp.maximum, jnp.max(p3, axis=0))
    mn = _fold(jnp.minimum, jnp.min(p3, axis=0))
    ep = jnp.exp2(p3 - mx[None])
    en = jnp.exp2(mn[None] - p3)
    zp = _fold(jnp.add, jnp.sum(ep, axis=0))
    zn = _fold(jnp.add, jnp.sum(en, axis=0))
    return ep, en, _recip(zp), _recip(zn)


LOPS = ((0, 3, 1), (2, 3, 1), (0, None, 0), (3, None, 0), (0, 1, 1), (2, 0, -1), (1, 3, -1))
ROPS = ((0, 3, 1), (0, None, 0), (1, 3, -1), (2, 0, -1), (3, None, 0), (0, 1, 1), (2, 3, 1))
ORDER = (2, 4, 1, 3, 0, 6, 5)
STEPS = ((2, 4), (1, 3), (0, 6), (5,))


def _lin(a, b, s):
    return a + b if s > 0 else a - b


def _ops7(table, q):
    return [q[a] if b is None else _lin(q[a], q[b], s) for a, b, s in table]


def _op1(table, k, q):
    a, b, s = table[k]
    if b is None:
        return q(a)
    return _lin(q(a).astype(f32), q(b).astype(f32), s).astype(bf16)


def _ops2(table, k1, blk, groups, fence):
    a, b, s = table[k1]
    out = [None] * 7
    for grp in groups:
        sub = {}

        def get(n2):
            if n2 not in sub:
                v = blk(a, n2).astype(f32)
                if b is not None:
                    v = _lin(v, blk(b, n2).astype(f32), s)
                sub[n2] = v
            return sub[n2]

        for k2 in grp:
            a2, b2, s2 = table[k2]
            if b is None and b2 is None:
                out[k2] = blk(a, a2)
            else:
                out[k2] = (get(a2) if b2 is None else _lin(get(a2), get(b2), s2)).astype(bf16)
        fence()
    return out


def _c11(m):
    return ((m[3] - m[4]) + m[0]) + m[6]


def _c12(m):
    return m[2] + m[4]


def _c21(m):
    return m[1] + m[3]


def _c22(m):
    return ((m[2] - m[1]) + m[0]) + m[5]


def _c11_late(m):
    return ((m[6] + m[0]) + m[3]) - m[4]


def _c22_late(m):
    return ((m[5] + m[0]) + m[2]) - m[1]


CQ = (_c12, _c21, _c11, _c22)
QORDER = ((1, 0), (0, 1), (0, 0), (1, 1))


def _ops_t(lhs, w_ref, j, scale=None):
    top = _dot(lhs[2 * j], w_ref[j, :, 0:128], NT)
    bot = _dot(lhs[2 * j + 1], w_ref[j, :, 128:256], NT)
    if scale is not None:
        top, bot = top * scale, bot * scale
    return _ops7(ROPS, [top[:, 0:KH], bot[:, 0:KH], top[:, KH:D], bot[:, KH:D]])


def _iota2(shape):
    return lax.broadcasted_iota(jnp.int32, shape, 0), lax.broadcasted_iota(jnp.int32, shape, 1)


def _kernel(x_hbm, wqkv_hbm, wphi_hbm, wo_hbm, wg_hbm, wu_hbm, wd_hbm, gw_hbm,
            o_hbm,
            wphi_ref, gw_ref, x_ref, wq_ref, wk_ref, wv_ref, wo_ref, wg_ref, wu_ref, wd_ref, out_ref,
            fence_ref, xsem, wsem, osem, kvsem):
    def xcopy(i):
        return pltpu.make_async_copy(x_hbm.at[pl.ds(i * T, T), :], x_ref.at[pl.ds(i * T, T), :], xsem.at[i])

    def ocopy(i, p):
        r0, n = OPIECES[p]
        r = i * T + r0
        if not isinstance(i, int):
            r = pl.multiple_of(r, 128)
        return pltpu.make_async_copy(out_ref.at[pl.ds(r, n), :], o_hbm.at[pl.ds(r, n), :],
                                     osem.at[len(OPIECES) * i + p])

    def wkv_copy(j):
        return [pltpu.make_async_copy(wqkv_hbm.at[:, pl.ds(base + j * KH, KH)], dst.at[j], kvsem.at[n * 2 + j])
                for n, (base, dst) in enumerate(((D, wk_ref), (2 * D, wv_ref)))]

    c_wphi = pltpu.make_async_copy(wphi_hbm, wphi_ref, wsem.at[0])
    late_copies = [
        pltpu.make_async_copy(wqkv_hbm.at[:, pl.ds(0, D)], wq_ref, wsem.at[1]),
        pltpu.make_async_copy(wg_hbm, wg_ref, wsem.at[2]),
        pltpu.make_async_copy(wu_hbm, wu_ref, wsem.at[3]),
        pltpu.make_async_copy(wd_hbm, wd_ref, wsem.at[4]),
        pltpu.make_async_copy(wo_hbm, wo_ref, wsem.at[5]),
        pltpu.make_async_copy(gw_hbm, gw_ref, wsem.at[6]),
    ]

    def fence():
        fence_ref[...] = jnp.zeros((8, 128), f32)

    c_wphi.start()
    for cp in wkv_copy(0):
        cp.start(priority=1)
    xcopy(0).start(priority=1)

    r, c = _iota2((H, D))
    sel = jnp.where(r == (c >> 4), 1.0, 0.0).astype(bf16)
    r, c = _iota2((256, D))
    m1 = (r >> 4) == (c & 15)
    r, c = _iota2((128, 256))
    rsel = jnp.where(((r & 63) >> 2) == (c & 15), 1.0, 0.0).astype(bf16)
    r, c = _iota2((128, D))
    m2 = ((r >> 6) * 4 + (r & 3)) == ((c >> 4) & 7)
    r, c = _iota2((128, 128))
    eye = jnp.where(r == c, 1.0, 0.0).astype(bf16)

    c_wphi.wait()
    for cp in wkv_copy(1):
        cp.start(priority=1)
    xcopy(1).start(priority=1)
    t1 = jnp.where(m1, _dot(wphi_ref[...], sel), 0.0).astype(bf16)
    ball = jnp.where(m2, _dot(rsel, t1), 0.0).astype(bf16)
    bjs = [ball[:, j * 128:(j + 1) * 128] for j in range(4)]

    skv = {}

    def prep_kv(j):
        ko = _ops_t(bjs, wk_ref, j, LOG2E)
        vo = _ops_t([eye] * 4, wv_ref, j)
        for k in range(7):
            for t in range(2):
                rows = slice(t * 64, (t + 1) * 64)
                skv[(k, 2 * j + t)] = jnp.concatenate([ko[k][rows], vo[k][rows]], axis=0).astype(bf16)

    for cp in wkv_copy(0):
        cp.wait()
    prep_kv(0)

    kv = [None] * NG
    zacc = [None] * NG

    def acc(lst, g, v):
        lst[g] = v if lst[g] is None else lst[g] + v

    def x_op(row0, k):
        def q(n):
            return x_ref[pl.ds(row0 + (n // 2) * TH, TH), (n % 2) * KH:(n % 2 + 1) * KH]
        s = _op1(LOPS, k, q)
        fence()
        return s

    def kv_piece(q, gl, ch, m):
        g = QORDER[q][0] * 4 + gl
        c = CQ[q]([None if t is None else t[:, ch * 128:(ch + 1) * 128] for t in m])
        ep, en, rp, rn = _softmax_pair(c[0:64, :])
        ph = jnp.concatenate([(ep * rp[None]).reshape(64, 128), (en * rn[None]).reshape(64, 128)], axis=0)
        acc(zacc, g, ph)
        acc(kv, g, _dot(c[64:128, :].astype(bf16), ph.astype(bf16), NT))

    pending = []

    def drain(n):
        for _ in range(min(n, len(pending))):
            kv_piece(*pending.pop(0))

    wqt, kvt, zbc = [None] * 4, [None] * NG, [None] * NG
    wops = {}

    def rhs_op(first, k, name, quads, rows, cols):
        if first:
            def q(n):
                ref, r0, c0 = quads[n]
                return ref[r0:r0 + rows, c0:c0 + cols]
            wops[(name, k)] = _op1(ROPS, k, q)
            fence()
        return wops[(name, k)]

    wd_q = ((wd_ref, 0, 0), (wd_ref, 0, KH), (wd_ref, FH, 0), (wd_ref, FH, KH))
    wo_q = ((wo_ref, 0, 0), (wo_ref, 0, KH), (wo_ref, KH, 0), (wo_ref, KH, KH))
    w_refs = (wg_ref, wu_ref)

    def phase_b(i, first, hook=None):
        row0 = i * T if first else pl.multiple_of(i * T, T)

        pq, ot = {}, {}

        def pq_piece(p):
            b, ch = p % 4, p // 4
            pq[p] = _dot(wqt[b], x_ref[pl.ds(row0 + ch * 128, 128), :], NT)

        def q_piece(p):
            b, ch = p % 4, p // 4
            o2 = []
            for gl in range(2):
                g = 2 * b + gl
                ep, en, rp, rn = _softmax_pair(pq[p][gl * 64:(gl + 1) * 64, :])
                dp = jnp.sum(ep * zbc[g][0:64].reshape(8, 8, 128), axis=0)
                dn = jnp.sum(en * zbc[g][64:128].reshape(8, 8, 128), axis=0)
                den = _fold(jnp.add, dp * rp + dn * rn) + 1e-6
                rd = 1.0 / den
                php = (ep * (rp * rd)[None]).reshape(64, 128)
                phn = (en * (rn * rd)[None]).reshape(64, 128)
                ph = jnp.concatenate([php, phn], axis=0).astype(bf16)
                o2.append(_dot(kvt[g], ph))
            ot[(b, ch)] = jnp.concatenate(o2, axis=0).T

        def oq(half, cw):
            return jnp.concatenate([jnp.concatenate([ot[(cw, ch)], ot[(cw + 2, ch)]], axis=1)
                                    for ch in (2 * half, 2 * half + 1)], axis=0)

        hc = [[None] * 14 for _ in range(4)]

        rm = [None] * 7
        for k in ORDER:
            xk = x_op(row0, k)
            rm[k] = jnp.concatenate(
                [_dot(xk, rhs_op(first, k, ('rem', mat),
                                 [(w_refs[mat], (n // 2) * KH, ((n % 2) * 7 + 6) * 128) for n in range(4)], KH, 128))
                 for mat in range(2)], axis=1)
        for n, cf in enumerate((_c11, _c12, _c21, _c22)):
            gu = cf(rm)
            hr = gu[:, 0:128] * gu[:, 128:256]
            for r2 in range(2):
                hc[(n // 2) * 2 + r2][(n % 2) * 7 + 6] = hr[r2 * TQ:(r2 + 1) * TQ, :]
        if hook is not None:
            hook()

        def xblk(n1, n2):
            r0 = (n1 // 2) * TH + (n2 // 2) * TQ
            c0 = (n1 % 2) * KH + (n2 % 2) * 128
            return x_ref[pl.ds(row0 + r0, TQ), c0:c0 + 128]

        step = 0
        x2 = [None] * 7
        for c in range(3):
            inner = [[None] * 7, [None] * 7]
            for k1 in ORDER:
                for mat in range(2):
                    def wblk(n1, n2):
                        r0 = (n1 // 2) * KH + (n2 // 2) * 128
                        c0 = ((n1 % 2) * 7 + (n2 % 2) * 3 + c) * 128
                        return w_refs[mat][r0:r0 + 128, c0:c0 + 128]
                    if 0 <= step - P0 < 16:
                        pq_piece(step - P0)
                    if c == 0 and mat == 0:
                        x2[k1] = _ops2(LOPS, k1, xblk, (ORDER,), fence)
                    if first:
                        wops[(c, mat, k1)] = _ops2(ROPS, k1, wblk, STEPS, fence)
                    m = [None] * 7
                    for k2 in ORDER:
                        m[k2] = _dot(x2[k1][k2], wops[(c, mat, k1)][k2])
                    inner[mat][k1] = [_c11(m), _c12(m), _c21(m), _c22(m)]
                    if 0 <= step - P0 - PLAG < 16:
                        q_piece(step - P0 - PLAG)
                    step += 1
            for n, cf in enumerate((_c11_late, _c12, _c21, _c22_late)):
                for sq in range(4):
                    g_, u_ = [cf([inner[mat][k1][sq] for k1 in range(7)]) for mat in range(2)]
                    hc[(n // 2) * 2 + sq // 2][(n % 2) * 7 + (sq % 2) * 3 + c] = g_ * u_

        h_top = jnp.concatenate([jnp.concatenate(hc[0], axis=1), jnp.concatenate(hc[1], axis=1)], axis=0)
        h_bot = jnp.concatenate([jnp.concatenate(hc[2], axis=1), jnp.concatenate(hc[3], axis=1)], axis=0)

        x = x_ref[pl.ds(row0, T), :]
        gwf = gw_ref[...].astype(f32)
        xg = x[:, 0:128].astype(f32) * gwf[0:1, :]
        for c in range(1, 4):
            xg = xg + x[:, c * 128:(c + 1) * 128].astype(f32) * gwf[c:c + 1, :]
        gate = jax.nn.sigmoid(jnp.sum(xg, axis=1, keepdims=True))
        g_t, g_b = gate[0:TH], gate[TH:T]

        ol = [t.astype(bf16) for t in _ops7(LOPS, [oq(0, 0), oq(0, 1), oq(1, 0), oq(1, 1)])]
        am = [None] * 7
        for k in ORDER:
            am[k] = _dot(ol[k], rhs_op(first, k, 'wo', wo_q, KH, KH))

        hl = [t.astype(bf16) for t in _ops7(LOPS, [h_top[:, 0:FH], h_top[:, FH:F], h_bot[:, 0:FH], h_bot[:, FH:F]])]
        bm = [None] * 7

        def down(k):
            bm[k] = _dot(hl[k], rhs_op(first, k, 'wd', wd_q, FH, KH))

        def emit(cf, gq, r0, c0):
            out_ref[pl.ds(row0 + r0, TH), c0:c0 + KH] = (gq * cf(am) + (1.0 - gq) * cf(bm)).astype(out_ref.dtype)

        down(2)
        down(4)
        emit(_c12, g_t, 0, KH)
        down(3)
        down(0)
        down(6)
        emit(_c11, g_t, 0, 0)
        ocopy(i, 0).start()
        down(1)
        emit(_c21, g_b, TH, 0)
        r5 = rhs_op(first, 5, 'wd', wd_q, FH, KH)
        for p in range(1, len(OPIECES)):
            r0, n = OPIECES[p][0] - TH, OPIECES[p][1]
            rows = slice(r0, r0 + n)
            bp = [None if m is None else m[rows] for m in bm]
            bp[5] = _dot(hl[5][rows], r5)
            res = g_b[rows] * _c22([m[rows] for m in am]) + (1.0 - g_b[rows]) * _c22(bp)
            out_ref[pl.ds(row0 + TH + r0, n), KH:D] = res.astype(out_ref.dtype)
            ocopy(i, p).start()

    xcopy(0).wait()
    for cp in [xcopy(2), xcopy(3)] + late_copies:
        cp.start(priority=1)

    x1 = [None] * 7
    for i in range(NB):
        for gl in range(4):
            if (i, gl) == (0, 2):
                for cp in wkv_copy(1):
                    cp.wait()
                xcopy(1).wait()
                prep_kv(1)
            if (i, gl) == (2, 0):
                xcopy(2).wait()
                xcopy(3).wait()
            m = [None] * 7
            for q in range(4):
                for k in STEPS[q]:
                    if gl == 0:
                        x1[k] = x_op(i * T, k)
                    m[k] = _dot(skv[(k, gl)], x1[k], NT)
                    drain(min(2 if len(pending) > LAG + 2 else 1, len(pending) - LAG))
                pending.extend((q, gl, ch, list(m)) for ch in range(TH // 128))

    for cp in late_copies:
        cp.wait()
    for ob in range(4):
        wqt[(ob // 2) + 2 * (ob % 2)] = (
            _dot(bjs[ob], wq_ref[:, ob * 128:(ob + 1) * 128], NT) * LOG2E).astype(bf16)

    def finish_a():
        drain(len(pending))
        rr, cc = _iota2((64, 128))
        same_head = (rr >> 4) == (cc & 3)
        for g in range(NG):
            kvt[g] = jnp.where(same_head, kv[g], 0.0).astype(bf16)
            zbc[g] = jnp.broadcast_to(jnp.sum(zacc[g], axis=1, keepdims=True), (128, 128))

    phase_b(0, True, finish_a)

    def body(i, carry):
        phase_b(i, False)
        return carry

    lax.fori_loop(1, NB, body, 0)
    for i in range(NB):
        for p in range(len(OPIECES)):
            ocopy(i, p).wait()


@jax.jit
def pallas_gated_mix__linear_kernel_hedgehog__glu_gated_bilinear__prompt_kernel(
    A_x: jax.Array,
    A_wqkv: jax.Array,
    A_w_phi: jax.Array,
    A_wo: jax.Array,
    B_x: jax.Array,
    B_w_gate: jax.Array,
    B_w_up: jax.Array,
    B_w_down: jax.Array,
    gate_w: jax.Array,
):
    del B_x
    x = A_x.reshape(S, D)
    wphi = jnp.transpose(A_w_phi, (1, 2, 0)).reshape(DH * DH, H)
    gw = gate_w.reshape(4, 128)

    hbm = pl.BlockSpec(memory_space=pl.ANY)

    out = pl.pallas_call(
        _kernel,
        in_specs=[hbm] * 8,
        out_specs=hbm,
        out_shape=jax.ShapeDtypeStruct((S, D), A_x.dtype),
        scratch_shapes=[
            pltpu.VMEM((DH * DH, H), bf16),
            pltpu.VMEM((4, 128), bf16),
            pltpu.VMEM((S, D), bf16),
            pltpu.VMEM((D, D), bf16),
            pltpu.VMEM((2, D, KH), bf16),
            pltpu.VMEM((2, D, KH), bf16),
            pltpu.VMEM((D, D), bf16),
            pltpu.VMEM((D, F), bf16),
            pltpu.VMEM((D, F), bf16),
            pltpu.VMEM((F, D), bf16),
            pltpu.VMEM((S, D), bf16),
            pltpu.VMEM((8, 128), f32),
            pltpu.SemaphoreType.DMA((NB,)),
            pltpu.SemaphoreType.DMA((7,)),
            pltpu.SemaphoreType.DMA((len(OPIECES) * NB,)),
            pltpu.SemaphoreType.DMA((4,)),
        ],
        compiler_params=pltpu.CompilerParams(
            vmem_limit_bytes=100 * 1024 * 1024,
        ),
    )(x, A_wqkv, wphi, A_wo, B_w_gate, B_w_up, B_w_down, gw)
    return out.reshape(1, S, D)
```

```python
import jax
import jax.numpy as jnp
from jax import lax
import jax.experimental.pallas as pl
import jax.experimental.pallas.tpu as pltpu

S, D, H, DH, F = 2048, 512, 32, 16, 1792
NG = 8
T = 512
NB = S // T
TH, TQ = T // 2, T // 4
KH, FH = D // 2, F // 2
LAG = 3
P0, PLAG = 14, 2
OPIECES = ((0, TH), (TH, 128), (TH + 128, 128))
LOG2E = 1.4426950408889634

f32 = jnp.float32
bf16 = jnp.bfloat16
NT = (((1,), (1,)), ((), ()))
NN = (((1,), (0,)), ((), ()))


def _dot(a, b, dims=NN):
    return lax.dot_general(a, b, dims, preferred_element_type=f32)


def _recip(z):
    r = pl.reciprocal(z, approx=True)
    return r * (2.0 - z * r)


def _fold(op, r):
    return op(r, pltpu.roll(r, 4, 0))


def _softmax_pair(p):
    p3 = p.reshape(8, 8, p.shape[-1])
    mx = _fold(jnp.maximum, jnp.max(p3, axis=0))
    mn = _fold(jnp.minimum, jnp.min(p3, axis=0))
    ep = jnp.exp2(p3 - mx[None])
    en = jnp.exp2(mn[None] - p3)
    zp = _fold(jnp.add, jnp.sum(ep, axis=0))
    zn = _fold(jnp.add, jnp.sum(en, axis=0))
    return ep, en, _recip(zp), _recip(zn)


LOPS = ((0, 3, 1), (2, 3, 1), (0, None, 0), (3, None, 0), (0, 1, 1), (2, 0, -1), (1, 3, -1))
ROPS = ((0, 3, 1), (0, None, 0), (1, 3, -1), (2, 0, -1), (3, None, 0), (0, 1, 1), (2, 3, 1))
ORDER = (2, 4, 1, 3, 0, 6, 5)
STEPS = ((2, 4), (1, 3), (0, 6), (5,))


def _lin(a, b, s):
    return a + b if s > 0 else a - b


def _ops7(table, q):
    return [q[a] if b is None else _lin(q[a], q[b], s) for a, b, s in table]


def _op1(table, k, q):
    a, b, s = table[k]
    if b is None:
        return q(a)
    return _lin(q(a).astype(f32), q(b).astype(f32), s).astype(bf16)


def _ops2(table, k1, blk, groups, fence):
    a, b, s = table[k1]
    out = [None] * 7
    for grp in groups:
        sub = {}

        def get(n2):
            if n2 not in sub:
                v = blk(a, n2).astype(f32)
                if b is not None:
                    v = _lin(v, blk(b, n2).astype(f32), s)
                sub[n2] = v
            return sub[n2]

        for k2 in grp:
            a2, b2, s2 = table[k2]
            if b is None and b2 is None:
                out[k2] = blk(a, a2)
            else:
                out[k2] = (get(a2) if b2 is None else _lin(get(a2), get(b2), s2)).astype(bf16)
        fence()
    return out


def _c11(m):
    return ((m[3] - m[4]) + m[0]) + m[6]


def _c12(m):
    return m[2] + m[4]


def _c21(m):
    return m[1] + m[3]


def _c22(m):
    return ((m[2] - m[1]) + m[0]) + m[5]


def _c11_late(m):
    return ((m[6] + m[0]) + m[3]) - m[4]


def _c22_late(m):
    return ((m[5] + m[0]) + m[2]) - m[1]


CQ = (_c12, _c21, _c11, _c22)
QORDER = ((1, 0), (0, 1), (0, 0), (1, 1))


def _ops_t(lhs, w_ref, j, scale=None):
    top = _dot(lhs[2 * j], w_ref[j, :, 0:128], NT)
    bot = _dot(lhs[2 * j + 1], w_ref[j, :, 128:256], NT)
    if scale is not None:
        top, bot = top * scale, bot * scale
    return _ops7(ROPS, [top[:, 0:KH], bot[:, 0:KH], top[:, KH:D], bot[:, KH:D]])


def _iota2(shape):
    return lax.broadcasted_iota(jnp.int32, shape, 0), lax.broadcasted_iota(jnp.int32, shape, 1)


def _kernel(x_hbm, wqkv_hbm, wphi_hbm, wo_hbm, wg_hbm, wu_hbm, wd_hbm, gw_hbm,
            o_hbm,
            wphi_ref, gw_ref, x_ref, wq_ref, wk_ref, wv_ref, wo_ref, wg_ref, wu_ref, wd_ref, out_ref,
            fence_ref, xsem, wsem, osem, kvsem):
    def xcopy(i):
        return pltpu.make_async_copy(x_hbm.at[pl.ds(i * T, T), :], x_ref.at[pl.ds(i * T, T), :], xsem.at[i])

    def ocopy(i, p):
        r0, n = OPIECES[p]
        r = i * T + r0
        if not isinstance(i, int):
            r = pl.multiple_of(r, 128)
        return pltpu.make_async_copy(out_ref.at[pl.ds(r, n), :], o_hbm.at[pl.ds(r, n), :],
                                     osem.at[len(OPIECES) * i + p])

    def wkv_copy(j):
        return [pltpu.make_async_copy(wqkv_hbm.at[:, pl.ds(base + j * KH, KH)], dst.at[j], kvsem.at[n * 2 + j])
                for n, (base, dst) in enumerate(((D, wk_ref), (2 * D, wv_ref)))]

    c_wphi = pltpu.make_async_copy(wphi_hbm, wphi_ref, wsem.at[0])
    late_copies = [
        pltpu.make_async_copy(wqkv_hbm.at[:, pl.ds(0, D)], wq_ref, wsem.at[1]),
        pltpu.make_async_copy(wg_hbm, wg_ref, wsem.at[2]),
        pltpu.make_async_copy(wu_hbm, wu_ref, wsem.at[3]),
        pltpu.make_async_copy(wd_hbm, wd_ref, wsem.at[4]),
        pltpu.make_async_copy(wo_hbm, wo_ref, wsem.at[5]),
        pltpu.make_async_copy(gw_hbm, gw_ref, wsem.at[6]),
    ]

    def fence():
        fence_ref[...] = jnp.zeros((8, 128), f32)

    c_wphi.start()
    for cp in wkv_copy(0):
        cp.start(priority=1)

    r, c = _iota2((H, D))
    sel = jnp.where(r == (c >> 4), 1.0, 0.0).astype(bf16)
    r, c = _iota2((256, D))
    m1 = (r >> 4) == (c & 15)
    r, c = _iota2((128, 256))
    rsel = jnp.where(((r & 63) >> 2) == (c & 15), 1.0, 0.0).astype(bf16)
    r, c = _iota2((128, D))
    m2 = ((r >> 6) * 4 + (r & 3)) == ((c >> 4) & 7)
    r, c = _iota2((128, 128))
    eye = jnp.where(r == c, 1.0, 0.0).astype(bf16)

    c_wphi.wait()
    xcopy(0).start(priority=1)
    t1 = jnp.where(m1, _dot(wphi_ref[...], sel), 0.0).astype(bf16)
    ball = jnp.where(m2, _dot(rsel, t1), 0.0).astype(bf16)
    bjs = [ball[:, j * 128:(j + 1) * 128] for j in range(4)]

    skv = {}

    def prep_kv(j):
        ko = _ops_t(bjs, wk_ref, j, LOG2E)
        vo = _ops_t([eye] * 4, wv_ref, j)
        for k in range(7):
            for t in range(2):
                rows = slice(t * 64, (t + 1) * 64)
                skv[(k, 2 * j + t)] = jnp.concatenate([ko[k][rows], vo[k][rows]], axis=0).astype(bf16)

    for cp in wkv_copy(0):
        cp.wait()
    for cp in wkv_copy(1):
        cp.start(priority=1)
    xcopy(1).start(priority=1)
    prep_kv(0)

    kv = [None] * NG
    zacc = [None] * NG

    def acc(lst, g, v):
        lst[g] = v if lst[g] is None else lst[g] + v

    def x_op(row0, k):
        def q(n):
            return x_ref[pl.ds(row0 + (n // 2) * TH, TH), (n % 2) * KH:(n % 2 + 1) * KH]
        s = _op1(LOPS, k, q)
        fence()
        return s

    def kv_piece(q, gl, ch, m):
        g = QORDER[q][0] * 4 + gl
        c = CQ[q]([None if t is None else t[:, ch * 128:(ch + 1) * 128] for t in m])
        ep, en, rp, rn = _softmax_pair(c[0:64, :])
        ph = jnp.concatenate([(ep * rp[None]).reshape(64, 128), (en * rn[None]).reshape(64, 128)], axis=0)
        acc(zacc, g, ph)
        acc(kv, g, _dot(c[64:128, :].astype(bf16), ph.astype(bf16), NT))

    pending = []

    def drain(n):
        for _ in range(min(n, len(pending))):
            kv_piece(*pending.pop(0))

    wqt, kvt, zbc = [None] * 4, [None] * NG, [None] * NG
    wops = {}

    def rhs_op(first, k, name, quads, rows, cols):
        if first:
            def q(n):
                ref, r0, c0 = quads[n]
                return ref[r0:r0 + rows, c0:c0 + cols]
            wops[(name, k)] = _op1(ROPS, k, q)
            fence()
        return wops[(name, k)]

    wd_q = ((wd_ref, 0, 0), (wd_ref, 0, KH), (wd_ref, FH, 0), (wd_ref, FH, KH))
    wo_q = ((wo_ref, 0, 0), (wo_ref, 0, KH), (wo_ref, KH, 0), (wo_ref, KH, KH))
    w_refs = (wg_ref, wu_ref)

    def phase_b(i, first, hook=None):
        row0 = i * T if first else pl.multiple_of(i * T, T)

        pq, ot = {}, {}

        def pq_piece(p):
            b, ch = p % 4, p // 4
            pq[p] = _dot(wqt[b], x_ref[pl.ds(row0 + ch * 128, 128), :], NT)

        def q_piece(p):
            b, ch = p % 4, p // 4
            o2 = []
            for gl in range(2):
                g = 2 * b + gl
                ep, en, rp, rn = _softmax_pair(pq[p][gl * 64:(gl + 1) * 64, :])
                dp = jnp.sum(ep * zbc[g][0:64].reshape(8, 8, 128), axis=0)
                dn = jnp.sum(en * zbc[g][64:128].reshape(8, 8, 128), axis=0)
                den = _fold(jnp.add, dp * rp + dn * rn) + 1e-6
                rd = 1.0 / den
                php = (ep * (rp * rd)[None]).reshape(64, 128)
                phn = (en * (rn * rd)[None]).reshape(64, 128)
                ph = jnp.concatenate([php, phn], axis=0).astype(bf16)
                o2.append(_dot(kvt[g], ph))
            ot[(b, ch)] = jnp.concatenate(o2, axis=0).T

        def oq(half, cw):
            return jnp.concatenate([jnp.concatenate([ot[(cw, ch)], ot[(cw + 2, ch)]], axis=1)
                                    for ch in (2 * half, 2 * half + 1)], axis=0)

        hc = [[None] * 14 for _ in range(4)]

        rm = [None] * 7

        def rem_prod(k):
            xk = x_op(row0, k)
            rm[k] = jnp.concatenate(
                [_dot(xk, rhs_op(first, k, ('rem', mat),
                                 [(w_refs[mat], (n // 2) * KH, ((n % 2) * 7 + 6) * 128) for n in range(4)], KH, 128))
                 for mat in range(2)], axis=1)

        def rem_done():
            for n, cf in enumerate((_c11, _c12, _c21, _c22)):
                gu = cf(rm)
                hr = gu[:, 0:128] * gu[:, 128:256]
                for r2 in range(2):
                    hc[(n // 2) * 2 + r2][(n % 2) * 7 + 6] = hr[r2 * TQ:(r2 + 1) * TQ, :]

        def xblk(n1, n2):
            r0 = (n1 // 2) * TH + (n2 // 2) * TQ
            c0 = (n1 % 2) * KH + (n2 % 2) * 128
            return x_ref[pl.ds(row0 + r0, TQ), c0:c0 + 128]

        step = 0
        x2 = [None] * 7
        for c in range(3):
            inner = [[None] * 7, [None] * 7]
            for k1 in ORDER:
                if c == 0:
                    rem_prod(k1)
                    if k1 == ORDER[1] and hook is not None:
                        hook()
                for mat in range(2):
                    def wblk(n1, n2):
                        r0 = (n1 // 2) * KH + (n2 // 2) * 128
                        c0 = ((n1 % 2) * 7 + (n2 % 2) * 3 + c) * 128
                        return w_refs[mat][r0:r0 + 128, c0:c0 + 128]
                    if 0 <= step - P0 < 16:
                        pq_piece(step - P0)
                    if c == 0 and mat == 0:
                        x2[k1] = _ops2(LOPS, k1, xblk, (ORDER,), fence)
                    if first:
                        wops[(c, mat, k1)] = _ops2(ROPS, k1, wblk, STEPS, fence)
                    m = [None] * 7
                    for k2 in ORDER:
                        m[k2] = _dot(x2[k1][k2], wops[(c, mat, k1)][k2])
                    inner[mat][k1] = [_c11(m), _c12(m), _c21(m), _c22(m)]
                    if 0 <= step - P0 - PLAG < 16:
                        q_piece(step - P0 - PLAG)
                    step += 1
            if c == 0:
                rem_done()
            for n, cf in enumerate((_c11_late, _c12, _c21, _c22_late)):
                for sq in range(4):
                    g_, u_ = [cf([inner[mat][k1][sq] for k1 in range(7)]) for mat in range(2)]
                    hc[(n // 2) * 2 + sq // 2][(n % 2) * 7 + (sq % 2) * 3 + c] = g_ * u_

        h_top = jnp.concatenate([jnp.concatenate(hc[0], axis=1), jnp.concatenate(hc[1], axis=1)], axis=0)
        h_bot = jnp.concatenate([jnp.concatenate(hc[2], axis=1), jnp.concatenate(hc[3], axis=1)], axis=0)

        x = x_ref[pl.ds(row0, T), :]
        gwf = gw_ref[...].astype(f32)
        xg = x[:, 0:128].astype(f32) * gwf[0:1, :]
        for c in range(1, 4):
            xg = xg + x[:, c * 128:(c + 1) * 128].astype(f32) * gwf[c:c + 1, :]
        gate = jax.nn.sigmoid(jnp.sum(xg, axis=1, keepdims=True))
        g_t, g_b = gate[0:TH], gate[TH:T]

        ol = [t.astype(bf16) for t in _ops7(LOPS, [oq(0, 0), oq(0, 1), oq(1, 0), oq(1, 1)])]
        am = [None] * 7
        for k in ORDER:
            am[k] = _dot(ol[k], rhs_op(first, k, 'wo', wo_q, KH, KH))

        hl = [t.astype(bf16) for t in _ops7(LOPS, [h_top[:, 0:FH], h_top[:, FH:F], h_bot[:, 0:FH], h_bot[:, FH:F]])]
        bm = [None] * 7

        def down(k):
            bm[k] = _dot(hl[k], rhs_op(first, k, 'wd', wd_q, FH, KH))

        def emit(cf, gq, r0, c0):
            out_ref[pl.ds(row0 + r0, TH), c0:c0 + KH] = (gq * cf(am) + (1.0 - gq) * cf(bm)).astype(out_ref.dtype)

        down(2)
        down(4)
        emit(_c12, g_t, 0, KH)
        down(3)
        down(0)
        down(6)
        emit(_c11, g_t, 0, 0)
        ocopy(i, 0).start()
        down(1)
        emit(_c21, g_b, TH, 0)
        r5 = rhs_op(first, 5, 'wd', wd_q, FH, KH)
        for p in range(1, len(OPIECES)):
            r0, n = OPIECES[p][0] - TH, OPIECES[p][1]
            rows = slice(r0, r0 + n)
            bp = [None if m is None else m[rows] for m in bm]
            bp[5] = _dot(hl[5][rows], r5)
            res = g_b[rows] * _c22([m[rows] for m in am]) + (1.0 - g_b[rows]) * _c22(bp)
            out_ref[pl.ds(row0 + TH + r0, n), KH:D] = res.astype(out_ref.dtype)
            ocopy(i, p).start()

    xcopy(0).wait()
    for cp in [xcopy(2), xcopy(3)] + late_copies:
        cp.start(priority=1)

    x1 = [None] * 7
    for i in range(NB):
        for gl in range(4):
            if (i, gl) == (0, 2):
                for cp in wkv_copy(1):
                    cp.wait()
                xcopy(1).wait()
                prep_kv(1)
            if (i, gl) == (2, 0):
                xcopy(2).wait()
                xcopy(3).wait()
            m = [None] * 7
            for q in range(4):
                for k in STEPS[q]:
                    if gl == 0:
                        x1[k] = x_op(i * T, k)
                    m[k] = _dot(skv[(k, gl)], x1[k], NT)
                    drain(min(2 if len(pending) > LAG + 2 else 1, len(pending) - LAG))
                pending.extend((q, gl, ch, list(m)) for ch in range(TH // 128))

    for cp in late_copies:
        cp.wait()
    for ob in range(4):
        wqt[(ob // 2) + 2 * (ob % 2)] = (
            _dot(bjs[ob], wq_ref[:, ob * 128:(ob + 1) * 128], NT) * LOG2E).astype(bf16)

    def finish_a():
        drain(len(pending))
        rr, cc = _iota2((64, 128))
        same_head = (rr >> 4) == (cc & 3)
        for g in range(NG):
            kvt[g] = jnp.where(same_head, kv[g], 0.0).astype(bf16)
            zbc[g] = jnp.broadcast_to(jnp.sum(zacc[g], axis=1, keepdims=True), (128, 128))

    phase_b(0, True, finish_a)

    def body(i, carry):
        phase_b(i, False)
        return carry

    lax.fori_loop(1, NB, body, 0)
    for i in range(NB):
        for p in range(len(OPIECES)):
            ocopy(i, p).wait()


@jax.jit
def pallas_gated_mix__linear_kernel_hedgehog__glu_gated_bilinear__prompt_kernel(
    A_x: jax.Array,
    A_wqkv: jax.Array,
    A_w_phi: jax.Array,
    A_wo: jax.Array,
    B_x: jax.Array,
    B_w_gate: jax.Array,
    B_w_up: jax.Array,
    B_w_down: jax.Array,
    gate_w: jax.Array,
):
    del B_x
    x = A_x.reshape(S, D)
    wphi = jnp.transpose(A_w_phi, (1, 2, 0)).reshape(DH * DH, H)
    gw = gate_w.reshape(4, 128)

    hbm = pl.BlockSpec(memory_space=pl.ANY)

    out = pl.pallas_call(
        _kernel,
        in_specs=[hbm] * 8,
        out_specs=hbm,
        out_shape=jax.ShapeDtypeStruct((S, D), A_x.dtype),
        scratch_shapes=[
            pltpu.VMEM((DH * DH, H), bf16),
            pltpu.VMEM((4, 128), bf16),
            pltpu.VMEM((S, D), bf16),
            pltpu.VMEM((D, D), bf16),
            pltpu.VMEM((2, D, KH), bf16),
            pltpu.VMEM((2, D, KH), bf16),
            pltpu.VMEM((D, D), bf16),
            pltpu.VMEM((D, F), bf16),
            pltpu.VMEM((D, F), bf16),
            pltpu.VMEM((F, D), bf16),
            pltpu.VMEM((S, D), bf16),
            pltpu.VMEM((8, 128), f32),
            pltpu.SemaphoreType.DMA((NB,)),
            pltpu.SemaphoreType.DMA((7,)),
            pltpu.SemaphoreType.DMA((len(OPIECES) * NB,)),
            pltpu.SemaphoreType.DMA((4,)),
        ],
        compiler_params=pltpu.CompilerParams(
            vmem_limit_bytes=100 * 1024 * 1024,
        ),
    )(x, A_wqkv, wphi, A_wo, B_w_gate, B_w_up, B_w_down, gw)
    return out.reshape(1, S, D)
```

```python
import jax
import jax.numpy as jnp
from jax import lax
import jax.experimental.pallas as pl
import jax.experimental.pallas.tpu as pltpu

S, D, H, DH, F = 2048, 512, 32, 16, 1792
NG = 8
T = 512
NB = S // T
TH, TQ = T // 2, T // 4
KH, FH = D // 2, F // 2
LAG = 3
P0, PLAG = 14, 2
OPIECES = ((0, TH), (TH, 128), (TH + 128, 128))
LOG2E = 1.4426950408889634

f32 = jnp.float32
bf16 = jnp.bfloat16
NT = (((1,), (1,)), ((), ()))
NN = (((1,), (0,)), ((), ()))


def _dot(a, b, dims=NN):
    return lax.dot_general(a, b, dims, preferred_element_type=f32)


def _recip(z):
    r = pl.reciprocal(z, approx=True)
    return r * (2.0 - z * r)


def _fold(op, r):
    return op(r, pltpu.roll(r, 4, 0))


def _softmax_pair(p):
    p3 = p.reshape(8, 8, p.shape[-1])
    mx = _fold(jnp.maximum, jnp.max(p3, axis=0))
    mn = _fold(jnp.minimum, jnp.min(p3, axis=0))
    ep = jnp.exp2(p3 - mx[None])
    en = jnp.exp2(mn[None] - p3)
    zp = _fold(jnp.add, jnp.sum(ep, axis=0))
    zn = _fold(jnp.add, jnp.sum(en, axis=0))
    return ep, en, _recip(zp), _recip(zn)


LOPS = ((0, 3, 1), (2, 3, 1), (0, None, 0), (3, None, 0), (0, 1, 1), (2, 0, -1), (1, 3, -1))
ROPS = ((0, 3, 1), (0, None, 0), (1, 3, -1), (2, 0, -1), (3, None, 0), (0, 1, 1), (2, 3, 1))
ORDER = (2, 4, 1, 3, 0, 6, 5)
STEPS = ((2, 4), (1, 3), (0, 6), (5,))


def _lin(a, b, s):
    return a + b if s > 0 else a - b


def _ops7(table, q):
    return [q[a] if b is None else _lin(q[a], q[b], s) for a, b, s in table]


def _op1(table, k, q):
    a, b, s = table[k]
    if b is None:
        return q(a)
    return _lin(q(a).astype(f32), q(b).astype(f32), s).astype(bf16)


def _ops2(table, k1, blk, groups, fence):
    a, b, s = table[k1]
    out = [None] * 7
    for grp in groups:
        sub = {}

        def get(n2):
            if n2 not in sub:
                v = blk(a, n2).astype(f32)
                if b is not None:
                    v = _lin(v, blk(b, n2).astype(f32), s)
                sub[n2] = v
            return sub[n2]

        for k2 in grp:
            a2, b2, s2 = table[k2]
            if b is None and b2 is None:
                out[k2] = blk(a, a2)
            else:
                out[k2] = (get(a2) if b2 is None else _lin(get(a2), get(b2), s2)).astype(bf16)
        fence()
    return out


def _c11(m):
    return ((m[3] - m[4]) + m[0]) + m[6]


def _c12(m):
    return m[2] + m[4]


def _c21(m):
    return m[1] + m[3]


def _c22(m):
    return ((m[2] - m[1]) + m[0]) + m[5]


def _c11_late(m):
    return ((m[6] + m[0]) + m[3]) - m[4]


def _c22_late(m):
    return ((m[5] + m[0]) + m[2]) - m[1]


CQ = (_c12, _c21, _c11, _c22)
QORDER = ((1, 0), (0, 1), (0, 0), (1, 1))


def _ops_t(lhs, w_ref, j, scale=None):
    top = _dot(lhs[2 * j], w_ref[j, :, 0:128], NT)
    bot = _dot(lhs[2 * j + 1], w_ref[j, :, 128:256], NT)
    if scale is not None:
        top, bot = top * scale, bot * scale
    return _ops7(ROPS, [top[:, 0:KH], bot[:, 0:KH], top[:, KH:D], bot[:, KH:D]])


def _iota2(shape):
    return lax.broadcasted_iota(jnp.int32, shape, 0), lax.broadcasted_iota(jnp.int32, shape, 1)


def _kernel(x_hbm, wqkv_hbm, wphi_hbm, wo_hbm, wg_hbm, wu_hbm, wd_hbm, gw_hbm,
            o_hbm,
            wphi_ref, gw_ref, x_ref, wq_ref, wk_ref, wv_ref, wo_ref, wg_ref, wu_ref, wd_ref, out_ref,
            fence_ref, sem):
    XSEM = (1, 3, 4, 4)

    def xcopy(i):
        return pltpu.make_async_copy(x_hbm.at[pl.ds(i * T, T), :], x_ref.at[pl.ds(i * T, T), :], sem.at[XSEM[i]])

    def ocopy(i, p):
        r0, n = OPIECES[p]
        r = i * T + r0
        if not isinstance(i, int):
            r = pl.multiple_of(r, 128)
        return pltpu.make_async_copy(out_ref.at[pl.ds(r, n), :], o_hbm.at[pl.ds(r, n), :], sem.at[6])

    def wkv_copy(j):
        return [pltpu.make_async_copy(wqkv_hbm.at[:, pl.ds(base + j * KH, KH)], dst.at[j], sem.at[2 + j])
                for base, dst in ((D, wk_ref), (2 * D, wv_ref))]

    c_wphi = pltpu.make_async_copy(wphi_hbm, wphi_ref, sem.at[0])
    late_copies = [
        pltpu.make_async_copy(wqkv_hbm.at[:, pl.ds(0, D)], wq_ref, sem.at[5]),
        pltpu.make_async_copy(wg_hbm, wg_ref, sem.at[5]),
        pltpu.make_async_copy(wu_hbm, wu_ref, sem.at[5]),
        pltpu.make_async_copy(wd_hbm, wd_ref, sem.at[5]),
        pltpu.make_async_copy(wo_hbm, wo_ref, sem.at[5]),
        pltpu.make_async_copy(gw_hbm, gw_ref, sem.at[5]),
    ]

    def fence():
        fence_ref[...] = jnp.zeros((8, 128), f32)

    c_wphi.start()
    for cp in wkv_copy(0):
        cp.start(priority=1)

    r, c = _iota2((H, D))
    sel = jnp.where(r == (c >> 4), 1.0, 0.0).astype(bf16)
    r, c = _iota2((256, D))
    m1 = (r >> 4) == (c & 15)
    r, c = _iota2((128, 256))
    rsel = jnp.where(((r & 63) >> 2) == (c & 15), 1.0, 0.0).astype(bf16)
    r, c = _iota2((128, D))
    m2 = ((r >> 6) * 4 + (r & 3)) == ((c >> 4) & 7)
    r, c = _iota2((128, 128))
    eye = jnp.where(r == c, 1.0, 0.0).astype(bf16)

    c_wphi.wait()
    xcopy(0).start(priority=1)
    t1 = jnp.where(m1, _dot(wphi_ref[...], sel), 0.0).astype(bf16)
    ball = jnp.where(m2, _dot(rsel, t1), 0.0).astype(bf16)
    bjs = [ball[:, j * 128:(j + 1) * 128] for j in range(4)]

    skv = {}

    def prep_kv(j):
        ko = _ops_t(bjs, wk_ref, j, LOG2E)
        vo = _ops_t([eye] * 4, wv_ref, j)
        for k in range(7):
            for t in range(2):
                rows = slice(t * 64, (t + 1) * 64)
                skv[(k, 2 * j + t)] = jnp.concatenate([ko[k][rows], vo[k][rows]], axis=0).astype(bf16)

    for cp in wkv_copy(0):
        cp.wait()
    for cp in wkv_copy(1):
        cp.start(priority=1)
    xcopy(1).start(priority=1)
    prep_kv(0)

    kv = [None] * NG
    zacc = [None] * NG

    def acc(lst, g, v):
        lst[g] = v if lst[g] is None else lst[g] + v

    def x_op(row0, k):
        def q(n):
            return x_ref[pl.ds(row0 + (n // 2) * TH, TH), (n % 2) * KH:(n % 2 + 1) * KH]
        s = _op1(LOPS, k, q)
        fence()
        return s

    def kv_piece(q, gl, ch, m):
        g = QORDER[q][0] * 4 + gl
        c = CQ[q]([None if t is None else t[:, ch * 128:(ch + 1) * 128] for t in m])
        ep, en, rp, rn = _softmax_pair(c[0:64, :])
        ph = jnp.concatenate([(ep * rp[None]).reshape(64, 128), (en * rn[None]).reshape(64, 128)], axis=0)
        acc(zacc, g, ph)
        acc(kv, g, _dot(c[64:128, :].astype(bf16), ph.astype(bf16), NT))

    pending = []

    def drain(n):
        for _ in range(min(n, len(pending))):
            kv_piece(*pending.pop(0))

    wqt, kvt, zbc = [None] * 4, [None] * NG, [None] * NG
    wops = {}

    def rhs_op(first, k, name, quads, rows, cols):
        if first:
            def q(n):
                ref, r0, c0 = quads[n]
                return ref[r0:r0 + rows, c0:c0 + cols]
            wops[(name, k)] = _op1(ROPS, k, q)
            fence()
        return wops[(name, k)]

    wd_q = ((wd_ref, 0, 0), (wd_ref, 0, KH), (wd_ref, FH, 0), (wd_ref, FH, KH))
    wo_q = ((wo_ref, 0, 0), (wo_ref, 0, KH), (wo_ref, KH, 0), (wo_ref, KH, KH))
    w_refs = (wg_ref, wu_ref)

    def phase_b(i, first, hook=None):
        row0 = i * T if first else pl.multiple_of(i * T, T)

        pq, ot = {}, {}

        def pq_piece(p):
            b, ch = p % 4, p // 4
            pq[p] = _dot(wqt[b], x_ref[pl.ds(row0 + ch * 128, 128), :], NT)

        def q_piece(p):
            b, ch = p % 4, p // 4
            o2 = []
            for gl in range(2):
                g = 2 * b + gl
                ep, en, rp, rn = _softmax_pair(pq[p][gl * 64:(gl + 1) * 64, :])
                dp = jnp.sum(ep * zbc[g][0:64].reshape(8, 8, 128), axis=0)
                dn = jnp.sum(en * zbc[g][64:128].reshape(8, 8, 128), axis=0)
                den = _fold(jnp.add, dp * rp + dn * rn) + 1e-6
                rd = 1.0 / den
                php = (ep * (rp * rd)[None]).reshape(64, 128)
                phn = (en * (rn * rd)[None]).reshape(64, 128)
                ph = jnp.concatenate([php, phn], axis=0).astype(bf16)
                o2.append(_dot(kvt[g], ph))
            ot[(b, ch)] = jnp.concatenate(o2, axis=0).T

        def oq(half, cw):
            return jnp.concatenate([jnp.concatenate([ot[(cw, ch)], ot[(cw + 2, ch)]], axis=1)
                                    for ch in (2 * half, 2 * half + 1)], axis=0)

        hc = [[None] * 14 for _ in range(4)]

        rm = [None] * 7

        def rem_prod(k):
            xk = x_op(row0, k)
            rm[k] = jnp.concatenate(
                [_dot(xk, rhs_op(first, k, ('rem', mat),
                                 [(w_refs[mat], (n // 2) * KH, ((n % 2) * 7 + 6) * 128) for n in range(4)], KH, 128))
                 for mat in range(2)], axis=1)

        def rem_done():
            for n, cf in enumerate((_c11, _c12, _c21, _c22)):
                gu = cf(rm)
                hr = gu[:, 0:128] * gu[:, 128:256]
                for r2 in range(2):
                    hc[(n // 2) * 2 + r2][(n % 2) * 7 + 6] = hr[r2 * TQ:(r2 + 1) * TQ, :]

        def xblk(n1, n2):
            r0 = (n1 // 2) * TH + (n2 // 2) * TQ
            c0 = (n1 % 2) * KH + (n2 % 2) * 128
            return x_ref[pl.ds(row0 + r0, TQ), c0:c0 + 128]

        step = 0
        x2 = [None] * 7
        for c in range(3):
            inner = [[None] * 7, [None] * 7]
            for k1 in ORDER:
                if c == 0:
                    rem_prod(k1)
                    if k1 == ORDER[1] and hook is not None:
                        hook()
                for mat in range(2):
                    def wblk(n1, n2):
                        r0 = (n1 // 2) * KH + (n2 // 2) * 128
                        c0 = ((n1 % 2) * 7 + (n2 % 2) * 3 + c) * 128
                        return w_refs[mat][r0:r0 + 128, c0:c0 + 128]
                    if 0 <= step - P0 < 16:
                        pq_piece(step - P0)
                    if c == 0 and mat == 0:
                        x2[k1] = _ops2(LOPS, k1, xblk, (ORDER,), fence)
                    if first:
                        wops[(c, mat, k1)] = _ops2(ROPS, k1, wblk, STEPS, fence)
                    m = [None] * 7
                    for k2 in ORDER:
                        m[k2] = _dot(x2[k1][k2], wops[(c, mat, k1)][k2])
                    inner[mat][k1] = [_c11(m), _c12(m), _c21(m), _c22(m)]
                    if 0 <= step - P0 - PLAG < 16:
                        q_piece(step - P0 - PLAG)
                    step += 1
            if c == 0:
                rem_done()
            for n, cf in enumerate((_c11_late, _c12, _c21, _c22_late)):
                for sq in range(4):
                    g_, u_ = [cf([inner[mat][k1][sq] for k1 in range(7)]) for mat in range(2)]
                    hc[(n // 2) * 2 + sq // 2][(n % 2) * 7 + (sq % 2) * 3 + c] = g_ * u_

        h_top = jnp.concatenate([jnp.concatenate(hc[0], axis=1), jnp.concatenate(hc[1], axis=1)], axis=0)
        h_bot = jnp.concatenate([jnp.concatenate(hc[2], axis=1), jnp.concatenate(hc[3], axis=1)], axis=0)

        x = x_ref[pl.ds(row0, T), :]
        gwf = gw_ref[...].astype(f32)
        xg = x[:, 0:128].astype(f32) * gwf[0:1, :]
        for c in range(1, 4):
            xg = xg + x[:, c * 128:(c + 1) * 128].astype(f32) * gwf[c:c + 1, :]
        gate = jax.nn.sigmoid(jnp.sum(xg, axis=1, keepdims=True))
        g_t, g_b = gate[0:TH], gate[TH:T]

        ol = [t.astype(bf16) for t in _ops7(LOPS, [oq(0, 0), oq(0, 1), oq(1, 0), oq(1, 1)])]
        am = [None] * 7
        for k in ORDER:
            am[k] = _dot(ol[k], rhs_op(first, k, 'wo', wo_q, KH, KH))

        hl = [t.astype(bf16) for t in _ops7(LOPS, [h_top[:, 0:FH], h_top[:, FH:F], h_bot[:, 0:FH], h_bot[:, FH:F]])]
        bm = [None] * 7

        def down(k):
            bm[k] = _dot(hl[k], rhs_op(first, k, 'wd', wd_q, FH, KH))

        def emit(cf, gq, r0, c0):
            out_ref[pl.ds(row0 + r0, TH), c0:c0 + KH] = (gq * cf(am) + (1.0 - gq) * cf(bm)).astype(out_ref.dtype)

        down(2)
        down(4)
        emit(_c12, g_t, 0, KH)
        down(3)
        down(0)
        down(6)
        emit(_c11, g_t, 0, 0)
        ocopy(i, 0).start()
        down(1)
        emit(_c21, g_b, TH, 0)
        r5 = rhs_op(first, 5, 'wd', wd_q, FH, KH)
        for p in range(1, len(OPIECES)):
            r0, n = OPIECES[p][0] - TH, OPIECES[p][1]
            rows = slice(r0, r0 + n)
            bp = [None if m is None else m[rows] for m in bm]
            bp[5] = _dot(hl[5][rows], r5)
            res = g_b[rows] * _c22([m[rows] for m in am]) + (1.0 - g_b[rows]) * _c22(bp)
            out_ref[pl.ds(row0 + TH + r0, n), KH:D] = res.astype(out_ref.dtype)
            ocopy(i, p).start()

    xcopy(0).wait()
    for cp in [xcopy(2), xcopy(3)] + late_copies:
        cp.start(priority=1)

    x1 = [None] * 7
    for i in range(NB):
        for gl in range(4):
            if (i, gl) == (0, 2):
                for cp in wkv_copy(1):
                    cp.wait()
                xcopy(1).wait()
                prep_kv(1)
            if (i, gl) == (2, 0):
                xcopy(2).wait()
                xcopy(3).wait()
            m = [None] * 7
            for q in range(4):
                for k in STEPS[q]:
                    if gl == 0:
                        x1[k] = x_op(i * T, k)
                    m[k] = _dot(skv[(k, gl)], x1[k], NT)
                    drain(min(2 if len(pending) > LAG + 2 else 1, len(pending) - LAG))
                pending.extend((q, gl, ch, list(m)) for ch in range(TH // 128))

    for cp in late_copies:
        cp.wait()
    for ob in range(4):
        wqt[(ob // 2) + 2 * (ob % 2)] = (
            _dot(bjs[ob], wq_ref[:, ob * 128:(ob + 1) * 128], NT) * LOG2E).astype(bf16)

    def finish_a():
        drain(len(pending))
        rr, cc = _iota2((64, 128))
        same_head = (rr >> 4) == (cc & 3)
        for g in range(NG):
            kvt[g] = jnp.where(same_head, kv[g], 0.0).astype(bf16)
            zbc[g] = jnp.broadcast_to(jnp.sum(zacc[g], axis=1, keepdims=True), (128, 128))

    phase_b(0, True, finish_a)

    def body(i, carry):
        phase_b(i, False)
        return carry

    lax.fori_loop(1, NB, body, 0)
    for i in range(NB):
        for p in range(len(OPIECES)):
            ocopy(i, p).wait()


@jax.jit
def pallas_gated_mix__linear_kernel_hedgehog__glu_gated_bilinear__prompt_kernel(
    A_x: jax.Array,
    A_wqkv: jax.Array,
    A_w_phi: jax.Array,
    A_wo: jax.Array,
    B_x: jax.Array,
    B_w_gate: jax.Array,
    B_w_up: jax.Array,
    B_w_down: jax.Array,
    gate_w: jax.Array,
):
    del B_x
    x = A_x.reshape(S, D)
    wphi = jnp.transpose(A_w_phi, (1, 2, 0)).reshape(DH * DH, H)
    gw = gate_w.reshape(4, 128)

    hbm = pl.BlockSpec(memory_space=pl.ANY)

    out = pl.pallas_call(
        _kernel,
        in_specs=[hbm] * 8,
        out_specs=hbm,
        out_shape=jax.ShapeDtypeStruct((S, D), A_x.dtype),
        scratch_shapes=[
            pltpu.VMEM((DH * DH, H), bf16),
            pltpu.VMEM((4, 128), bf16),
            pltpu.VMEM((S, D), bf16),
            pltpu.VMEM((D, D), bf16),
            pltpu.VMEM((2, D, KH), bf16),
            pltpu.VMEM((2, D, KH), bf16),
            pltpu.VMEM((D, D), bf16),
            pltpu.VMEM((D, F), bf16),
            pltpu.VMEM((D, F), bf16),
            pltpu.VMEM((F, D), bf16),
            pltpu.VMEM((S, D), bf16),
            pltpu.VMEM((8, 128), f32),
            pltpu.SemaphoreType.DMA((7,)),
        ],
        compiler_params=pltpu.CompilerParams(
            vmem_limit_bytes=100 * 1024 * 1024,
        ),
    )(x, A_wqkv, wphi, A_wo, B_w_gate, B_w_up, B_w_down, gw)
    return out.reshape(1, S, D)
```
